```python
import os as _os
_os.environ.setdefault("JAX_PLATFORMS", "cpu")
import jax
import jax.numpy as jnp

def _softmax(x, axis=-1):
    return jax.nn.softmax(x, axis=axis)
def _gelu(x):
    return jax.nn.gelu(x, approximate=True)
def _silu(x):
    return jax.nn.silu(x)
def _sigmoid(x):
    return jax.nn.sigmoid(x)
def _layernorm(x, axis=-1, eps=1e-5):
    m = jnp.mean(x, axis=axis, keepdims=True)
    v = jnp.var(x, axis=axis, keepdims=True)
    return (x - m) / jnp.sqrt(v + eps)
def _scatter_add(tgt, idx, src, axis=0):
    return tgt.at[idx].add(src)
def _segment_sum(src, seg, n):
    return jax.ops.segment_sum(src, seg, n)
class _Rng:
    def __init__(self, key):
        self._k = key
    def _next(self):
        self._k, sub = jax.random.split(self._k)
        return sub
    def normal(self, shape):
        return jax.random.normal(self._next(), shape, dtype=jnp.bfloat16)
    def randint(self, lo, hi, shape):
        return jax.random.randint(self._next(), shape, lo, hi, dtype=jnp.int32)
    def uniform(self, shape, lo=0.0, hi=1.0):
        return jax.random.uniform(self._next(), shape, jnp.bfloat16, lo, hi)
    def permutation(self, n):
        return jax.random.permutation(self._next(), n)


kernel_name = 'concat_heads__spectral_gfnet__sliding_block__prompt'

def setup_inputs():
    _rng = _Rng(jax.random.key(int.from_bytes(__import__("os").urandom(4), "little")))
    _w = (lambda a: (lambda t: t.astype(jnp.bfloat16) if jnp.issubdtype(t.dtype, jnp.floating) else t)(jnp.asarray(a)))
    def _A_setup():
        B, S, D = 1, 2048, 640
        Df = D // 2 + 1
        return {
            "x": _w((lambda *s: _rng.normal(s) * 0.05)(B, S, D)),
            "w_r": _w((lambda *s: _rng.normal(s) * 0.4)(S, Df) * 0.02),
            "w_i": _w((lambda *s: _rng.normal(s) * 0.4)(S, Df) * 0.02),
        }
    _A_in = _A_setup()

    def _B_setup():
        B, S, D = 1, 2048, 640
        return {
            "x": _w((lambda *s: _rng.normal(s) * 0.2)(B, S, D)),
            "wqkv": _w((lambda *s: _rng.normal(s) * 0.2)(D, 3 * D)),
            "wo": _w((lambda *s: _rng.normal(s) * 0.05)(D, D)),
        }
    _B_in = _B_setup()

    return {
        "A_x": _A_in["x"],
        "A_w_r": _A_in["w_r"],
        "A_w_i": _A_in["w_i"],
        "B_x": _B_in["x"],
        "B_wqkv": _B_in["wqkv"],
        "B_wo": _B_in["wo"],
    }

def reference(A_x, A_w_r, A_w_i, B_x, B_wqkv, B_wo):
    def _A_ref(x, w_r, w_i):
        B, S, D = x.shape
        X = (lambda x, axes=(-2,-1): jnp.fft.rfft2(x.astype(jnp.float32), axes=axes))(x, axes=(-2, -1))
        W = w_r + 1j * w_i
        X = X * W
        y = (lambda x, s, axes=(-2,-1): jnp.fft.irfft2(x, s=s, axes=axes).astype(jnp.bfloat16))(X, (S, D), axes=(-2, -1))
        return y

    def _B_ref(x, wqkv, wo):
        B, S, D = x.shape
        H = 32; Dh = D // H; W = 256
        qkv = (lambda x, *d: x.transpose(*d))((x @ wqkv).reshape(B, S, 3, H, Dh), 2, 0, 3, 1, 4)
        q, k, v = qkv[0], qkv[1], qkv[2]
        scores = jnp.einsum("bhqd,bhkd->bhqk", q, k) * (Dh ** -0.5)
        idx = jnp.arange(S)
        mask = (idx[:, None] - idx[None, :] >= 0) & (idx[:, None] - idx[None, :] < W)
        scores = jnp.where(mask[None, None], scores, -1e9)
        p = _softmax(scores, axis=-1)
        o = jnp.einsum("bhqk,bhkd->bhqd", p, v)
        return (lambda x, *d: x.transpose(*d))(o, 0, 2, 1, 3).reshape(B, S, D) @ wo

    a = _A_ref(A_x, A_w_r, A_w_i)
    b = _B_ref(B_x, B_wqkv, B_wo)
    return jnp.concatenate([a, b], axis=-1)
```

```python
import numpy as np
S, D = 2048, 640
C1, C2 = np.cos(2*np.pi/5), np.cos(4*np.pi/5)
S1, S2 = np.sin(2*np.pi/5), np.sin(4*np.pi/5)
RHO = S2 / S1

def lane_layout():
    cls = [((0,1),38), ((0,2),13), ((1,0),38), ((1,2),13), ((2,0),13), ((2,1),13)]
    a_src = []; b_src = []
    for (a, b), n in cls:
        a_src += [a]*n; b_src += [b]*n
    a_src = np.array(a_src); b_src = np.array(b_src)
    c_src = np.full(128, -1)
    for l in range(128):
        a, b = a_src[l], b_src[l]
        if {a, b} == {1, 2}: c_src[l] = 0
        elif {a, b} == {0, 2}: c_src[l] = 1
    c_src[:13] = 2
    ks = np.arange(321)
    def assign(src, res):
        out = np.full(128, -1)
        for s in range(3):
            cand = [k for k in ks if k // 128 == s and (k % 5) in res]
            lanes = np.nonzero(src == s)[0]
            assert len(cand) == len(lanes), (s, len(cand), len(lanes))
            out[lanes] = cand
        return out
    kA = assign(a_src, (1, 4)); kB = assign(b_src, (2, 3)); kC = assign(c_src, (0,))
    gidx = np.zeros((3, 128), np.int32)
    for kk, src in ((kA, a_src), (kB, b_src), (kC, c_src)):
        for l in range(128):
            if kk[l] >= 0:
                gidx[src[l], l] = kk[l] - 128*src[l]
    return kA, kB, kC, a_src, b_src, c_src, gidx

def row_mats():
    kA, kB, kC, *_ = lane_layout()
    m2 = np.arange(128)[:, None]
    def cs(k):
        ang = 2*np.pi*m2*np.where(k >= 0, k, 0)[None, :]/D
        v = (k >= 0)[None, :]
        return np.cos(ang)*v, np.sin(ang)*v
    def fwd_pair(k, first):
        C, Sn = cs(k)
        sg = np.where(k % 5 == first, -1.0, 1.0)[None, :] * S1
        M = np.zeros((256, 256))
        M[:128, :128] = C; M[:128, 128:] = -Sn
        M[128:, :128] = sg*Sn; M[128:, 128:] = sg*C
        return M
    MA = fwd_pair(kA, 1); MB = fwd_pair(kB, 2)
    C, Sn = cs(kC)
    MC = np.concatenate([C, -Sn], axis=1)
    norm = 1.0/(S*D)
    def inv_pair(k, first):
        C, Sn = cs(k)
        w = 2.0*norm
        sg = np.where(k % 5 == first, 1.0, -1.0)[None, :] * S1
        N = np.zeros((256, 256))
        N[:128, :128] = (w*C).T; N[128:, :128] = (-w*Sn).T
        N[:128, 128:] = (w*sg*Sn).T; N[128:, 128:] = (w*sg*C).T
        return N
    NA = inv_pair(kA, 1); NB = inv_pair(kB, 2)
    w = np.where((kC == 0) | (kC == 320), 1.0, 2.0)[None, :]*norm
    NC = np.concatenate([(w*C).T, (-w*Sn).T], axis=0)
    return MA, MB, MC, NA, NB, NC

def col_mats():
    k2 = np.arange(64)[:, None]; n2 = np.arange(64)[None, :]
    Gf = np.zeros((32, 128, 128))
    for k1 in range(32):
        ang = -2*np.pi*((n2*(k1 + 32*k2)) % S)/S
        gr, gi = np.cos(ang), np.sin(ang)
        Gf[k1, :64, :64] = gr; Gf[k1, :64, 64:] = -gi
        Gf[k1, 64:, :64] = gi; Gf[k1, 64:, 64:] = gr
    Gi = Gf.transpose(0, 2, 1).copy()
    return Gf, Gi


import functools
import jax, jax.numpy as jnp, numpy as np
from jax.experimental import pallas as pl
from jax.experimental.pallas import tpu as pltpu

S, D = 2048, 640
BF = jnp.bfloat16; F32 = jnp.float32; U32 = jnp.uint32; I32 = jnp.int32
def dot(a, b): return jnp.dot(a, b, preferred_element_type=F32)
def bc(x, dt): return pltpu.bitcast(x, dt)
iota = jax.lax.broadcasted_iota
RHO = float(RHO); R54 = float(np.sqrt(5)/4); RT = float(np.sqrt(0.5))

def cmul_const(z, ang_num, ang_den, sign):
    x, y = z
    n = (ang_num * 8) % (8*ang_den)
    if ang_num % ang_den == 0: return z
    if (ang_num * 4) % ang_den == 0:
        q = ((ang_num * 4) // ang_den) % 4
        q = q if sign > 0 else (-q) % 4
        if q == 1: return (-y, x)
        if q == 2: return (-x, -y)
        if q == 3: return (y, -x)
    if (ang_num * 8) % ang_den == 0:
        o = ((ang_num * 8) // ang_den) % 8
        o = o if sign > 0 else (-o) % 8
        c = 1 if o in (1, 7) else -1
        d = 1 if o in (1, 3) else -1
        if c == 1 and d == 1: return ((x - y) * RT, (x + y) * RT)
        if c == 1 and d == -1: return ((x + y) * RT, (y - x) * RT)
        if c == -1 and d == 1: return ((x + y) * (-RT), (x - y) * RT)
        return ((y - x) * RT, (x + y) * (-RT))
    ang = sign * 2*np.pi*ang_num/ang_den
    c, d = float(np.cos(ang)), float(np.sin(ang))
    return (x*c - y*d, x*d + y*c)

def cadd(a, b): return (a[0]+b[0], a[1]+b[1])
def csub(a, b): return (a[0]-b[0], a[1]-b[1])
def rot(t, u, sign):
    if sign > 0:
        return (t[0]-u[1], t[1]+u[0]), (t[0]+u[1], t[1]-u[0])
    return (t[0]+u[1], t[1]-u[0]), (t[0]-u[1], t[1]+u[0])

def radix4(z, sign):
    t0, t1, t2, t3 = cadd(z[0], z[2]), csub(z[0], z[2]), cadd(z[1], z[3]), csub(z[1], z[3])
    s1, s3 = rot(t1, t3, sign)
    return [cadd(t0, t2), s1, csub(t0, t2), s3]

def radix8(z, sign):
    u = [cadd(z[b], z[b+4]) for b in range(4)]
    v = [csub(z[b], z[b+4]) for b in range(4)]
    ev = radix4(u, sign)
    v1 = cmul_const(v[1], 1, 8, sign); v3 = cmul_const(v[3], 3, 8, sign)
    t0, t1 = rot(v[0], v[2], sign)
    t2, t3 = cadd(v1, v3), csub(v1, v3)
    s1, s3 = rot(t1, t3, sign)
    od = [cadd(t0, t2), s1, csub(t0, t2), s3]
    out = []
    for j in range(4): out += [ev[j], od[j]]
    return out

def a_consts():
    kA, kB, kC, a_src, b_src, c_src, gidx = lane_layout()
    MA, MB, MC, NA, NB, NC = row_mats(); Gf, Gi = col_mats()
    M = np.concatenate([MA, MB, MC], 0).astype(BF)
    N = np.concatenate([NA, NB, np.concatenate([NC, np.zeros((256,128))], 1)], 0).astype(BF)
    gi8 = np.zeros((8,128), np.int32); gi8[:3] = gidx
    return M, N, Gf.astype(BF), Gi.astype(BF), gi8, (a_src, b_src, c_src)

def lane_sel_mask(src, s, lane8):
    m = None; l = 0
    while l < 128:
        if src[l] == s:
            r = l
            while r < 128 and src[r] == s: r += 1
            t = (lane8 >= l) & (lane8 < r)
            m = t if m is None else (m | t)
            l = r
        else: l += 1
    return m

class AParts:
    def __init__(self, xa_ref, wr_ref, wi_ref, M_ref, N_ref, Gf_ref, Gi_ref, gi_ref, Wp_ref, Sf_ref, Yb_ref, Rb_ref, ya_ref, srcs, out_dma):
        self.xa_ref, self.wr_ref, self.wi_ref, self.M_ref, self.N_ref = xa_ref, wr_ref, wi_ref, M_ref, N_ref
        self.Gf_ref, self.Gi_ref, self.gi_ref, self.Wp_ref, self.Sf_ref = Gf_ref, Gi_ref, gi_ref, Wp_ref, Sf_ref
        self.Yb_ref, self.Rb_ref, self.ya_ref, self.srcs, self.out_dma = Yb_ref, Rb_ref, ya_ref, srcs, out_dma
        self.Tf_ref = Sf_ref

    def wprep_pieces(self):
        s = self
        lane8 = iota(I32, (8,128), 1)
        a_src, b_src, c_src = s.srcs
        def piece(j, arr):
            def f():
                ref = (s.wr_ref, s.wi_ref)[arr]
                gidx = [jnp.broadcast_to(s.gi_ref[t:t+1, :], (8,128)) for t in range(3)]
                mA0, mA1 = lane_sel_mask(a_src,0,lane8), lane_sel_mask(a_src,1,lane8)
                mB0, mB1 = lane_sel_mask(b_src,0,lane8), lane_sel_mask(b_src,1,lane8)
                mC0, mC1 = lane_sel_mask(c_src,0,lane8), lane_sel_mask(c_src,1,lane8)
                cols = slice(128*j, 128*j+128)
                t2 = jnp.concatenate([ref[256:321, cols], jnp.zeros((63, 128), BF)], axis=0)
                tiles = [bc(ref[0:128, cols].T, U32), bc(ref[128:256, cols].T, U32), bc(t2.T, U32)]
                for v in range(8):
                    u = 8*j + v
                    g = [jnp.take_along_axis(tiles[t][8*v:8*v+8], gidx[t], axis=1) for t in range(3)]
                    pos = 17*(u//2) + 8*(u % 2)
                    s.Wp_ref[arr, 0, pos:pos+8, :] = jnp.where(mA0, g[0], jnp.where(mA1, g[1], g[2]))
                    s.Wp_ref[arr, 1, pos:pos+8, :] = jnp.where(mB0, g[0], jnp.where(mB1, g[1], g[2]))
                    s.Wp_ref[arr, 2, pos:pos+8, :] = jnp.where(mC0, g[0], jnp.where(mC1, g[1], g[2]))
            return f
        return [piece(j, arr) for j in range(16) for arr in range(2)]

    def f1_pieces(self):
        s = self
        def piece(b, g):
            def f():
                def xt(t):
                    return jnp.concatenate([s.xa_ref[64*(8*a+b)+16*g: 64*(8*a+b)+16*g+16, t*128:(t+1)*128] for a in range(4)], axis=0).astype(F32)
                T = [xt(t) for t in range(5)]
                p, q, r, w = T[1]+T[4], T[2]+T[3], T[1]-T[4], T[2]-T[3]
                u = p+q
                U0 = (T[0]+u).astype(BF)
                t1 = T[0] - 0.25*u; t2 = (p-q)*R54
                a1 = (t1+t2).astype(BF); a2 = (t1-t2).astype(BF)
                b1 = (r + RHO*w).astype(BF); b2 = (RHO*r - w).astype(BF)
                RA = dot(jnp.concatenate([a1, b1], axis=1), s.M_ref[0:256, :])
                RB = dot(jnp.concatenate([a2, b2], axis=1), s.M_ref[256:512, :])
                RC = dot(U0, s.M_ref[512:640, :])
                for P, R in enumerate((RA, RB, RC)):
                    z = [(R[16*a:16*a+16, 0:128], R[16*a:16*a+16, 128:256]) for a in range(4)]
                    Sx = radix4(z, -1)
                    for ka in range(4):
                        x, y = cmul_const(Sx[ka], b*ka, 32, -1)
                        s.Sf_ref[P, 0, ka, b, 16*g:16*g+16, :] = x
                        s.Sf_ref[P, 1, ka, b, 16*g:16*g+16, :] = y
            return f
        return [piece(b, g) for g in range(4) for b in range(8)]

    def f2_pieces(self):
        s = self
        def piece(ka, g, P):
            def f():
                z = [(s.Sf_ref[P, 0, ka, b, 16*g:16*g+16, :], s.Sf_ref[P, 1, ka, b, 16*g:16*g+16, :]) for b in range(8)]
                o = radix8(z, -1)
                for kb in range(8):
                    k1 = ka + 4*kb
                    s.Yb_ref[k1, P, 16*g:16*g+16, :] = o[kb][0].astype(BF)
                    s.Yb_ref[k1, P, 64+16*g:64+16*g+16, :] = o[kb][1].astype(BF)
            return f
        return [piece(ka, g, P) for ka in range(4) for P in range(3) for g in range(4)]

    def m_pieces(self):
        s = self
        def piece(be, P):
            def f():
                V = []
                for al in range(4):
                    k1 = be + 8*al
                    X = dot(s.Gf_ref[k1], s.Yb_ref[k1, P])
                    wr = s.Wp_ref[0, P, pl.ds(k1//2, 64, stride=17), :]
                    wi = s.Wp_ref[1, P, pl.ds(k1//2, 64, stride=17), :]
                    if k1 % 2 == 0:
                        wr = bc(wr << 16, F32); wi = bc(wi << 16, F32)
                    else:
                        wr = bc(wr & jnp.uint32(0xFFFF0000), F32); wi = bc(wi & jnp.uint32(0xFFFF0000), F32)
                    xr, xi = X[0:64], X[64:128]
                    Z = jnp.concatenate([xr*wr - xi*wi, xr*wi + xi*wr], axis=0).astype(BF)
                    Vv = dot(s.Gi_ref[k1], Z)
                    V.append((Vv[0:64], Vv[64:128]))
                Tn = radix4(V, +1)
                for na in range(4):
                    x, y = cmul_const(Tn[na], be*na, 32, +1)
                    s.Tf_ref[P, 0, na, be] = x
                    s.Tf_ref[P, 1, na, be] = y
            return f
        return [piece(be, P) for P in range(3) for be in range(8)]

    def i2_pieces(self):
        s = self
        def piece(na, g, P):
            def f():
                z = [(s.Tf_ref[P, 0, na, be, 16*g:16*g+16, :], s.Tf_ref[P, 1, na, be, 16*g:16*g+16, :]) for be in range(8)]
                o = radix8(z, +1)
                for nb in range(8):
                    n1 = na + 4*nb
                    s.Rb_ref[2*P, 64*n1+16*g:64*n1+16*g+16, :] = o[nb][0].astype(BF)
                    s.Rb_ref[2*P+1, 64*n1+16*g:64*n1+16*g+16, :] = o[nb][1].astype(BF)
            return f
        return [piece(na, g, P) for P in range(3) for na in range(4) for g in range(4)]

    def i1_pieces(self, R=128):
        s = self
        def piece(j):
            def f():
                rows = slice(R*j, R*(j+1))
                EA = dot(jnp.concatenate([s.Rb_ref[0, rows, :], s.Rb_ref[1, rows, :]], axis=1), s.N_ref[0:256, :])
                EB = dot(jnp.concatenate([s.Rb_ref[2, rows, :], s.Rb_ref[3, rows, :]], axis=1), s.N_ref[256:512, :])
                U0 = dot(jnp.concatenate([s.Rb_ref[4, rows, :], s.Rb_ref[5, rows, :]], axis=1), s.N_ref[512:768, 0:128])
                e1, f1, e2, f2 = EA[:, :128], EA[:, 128:], EB[:, :128], EB[:, 128:]
                u = e1+e2
                t1 = U0 - 0.25*u; t2 = (e1-e2)*R54
                al, be = t1+t2, t1-t2
                ga = f1 + RHO*f2; de = RHO*f1 - f2
                ys = [U0+u, al-ga, be-de, be+de, al+ga]
                for t in range(5):
                    s.ya_ref[rows, t*128:(t+1)*128] = ys[t].astype(BF)
                s.out_dma(j, R)
            return f
        return [piece(j) for j in range(S // R)]


H, DH, WIN = 32, 20, 256
NB = S // 128
NEG = -1e30
QSCALE = float((DH ** -0.5) * np.log2(np.e))
def nt_dot(a, b): return jax.lax.dot_general(a, b, (((1,), (1,)), ((), ())), preferred_element_type=F32)

def head_geom(h):
    c0 = DH*h; t = c0//128
    straddle = (c0+DH-1)//128 != t
    base = 128*t + (64 if straddle else 0)
    a = (c0//16)*16; off = c0 - a
    return c0, base, a, off

def merge_streams(streams):
    items = []
    for si, st in enumerate(streams):
        n = len(st)
        for j, f in enumerate(st):
            items.append(((j + 0.5) / n, si, j, f))
    items.sort(key=lambda t: (t[0], t[1]))
    for _, _, _, f in items: f()

def new_mask_const():
    j = np.arange(64)[:, None]; r = np.arange(128)[None, :]
    lo = (2*j <= r).astype(np.uint32) * np.uint32(0xFFFF)
    hi = (2*j + 1 <= r).astype(np.uint32) * np.uint32(0xFFFF0000)
    return (lo | hi).astype(np.uint32)

def full_kernel(xa_hbm, wr_hbm, wi_hbm, x_hbm, wqkv_hbm, wo_hbm, cst_hbm, M_hbm, N_hbm, Gf_hbm, Gi_hbm, o_hbm,
                xa_ref, wr_ref, wi_ref, M_ref, N_ref, Gf_ref, Gi_ref, Wp_ref, Sf_ref, Yb_ref, Rb_ref, ya_ref,
                x_ref, wqkv_ref, wo_ref, cst_ref, wT_ref, qT_ref, vT_ref, kw_ref, ks_ref, oT_ref, y_ref, sems,
                *, srcs, G=4, order="pipe3", plan=None):
    mk_ref = cst_ref.at[pl.ds(0, 64), :]
    gi_ref = cst_ref.at[pl.ds(64, 8), :].bitcast(I32)
    nsem = [0]
    def mk_copy(src, dst):
        c = pltpu.make_async_copy(src, dst, sems.at[nsem[0]]); nsem[0] += 1
        return c
    cp_w = [mk_copy(wqkv_hbm.at[:, pl.ds(640*j, 640)], wqkv_ref.at[:, pl.ds(640*j, 640)]) for j in (1, 0, 2)]
    cp_x = [mk_copy(x_hbm.at[pl.ds(r0, n), :], x_ref.at[pl.ds(r0, n), :]) for r0, n in ((0, 256), (256, 256), (512, 512), (1024, 1024))]
    x_chunk_of_block = [0, 0, 1, 1, 2, 2, 2, 2] + [3]*8
    cp_wo = mk_copy(wo_hbm, wo_ref)
    cp_cst = mk_copy(cst_hbm, cst_ref)
    cp_M = mk_copy(M_hbm, M_ref); cp_xa = mk_copy(xa_hbm, xa_ref)
    cp_wr = mk_copy(wr_hbm, wr_ref); cp_wi = mk_copy(wi_hbm, wi_ref)
    cp_Gf = mk_copy(Gf_hbm, Gf_ref); cp_Gi = mk_copy(Gi_hbm, Gi_ref); cp_N = mk_copy(N_hbm, N_ref)
    out_copies = []
    def a_out_dma(j, R):
        c = mk_copy(ya_ref.at[pl.ds(R*j, R), :], o_hbm.at[pl.ds(R*j, R), pl.ds(0, D)])
        c.start(); out_copies.append(c)

    sub8 = iota(I32, (8,128), 0); lane8 = iota(I32, (8,128), 1)
    zero8 = jnp.zeros((8,128), U32)

    def proj_pieces(i):
        rows = pl.ds(i*128, 128)
        ktiles = {}
        def kpiece(t):
            def f():
                kt = dot(x_ref[rows, :], wqkv_ref[:, 640 + t*128: 640 + (t+1)*128])
                ku = bc(kt.astype(BF), U32)
                kr = pltpu.roll(ku, 64, 1)
                kw_ref[2*t, pl.ds(i*64, 64), :] = ku
                ks_ref[2*t, pl.ds(i*64, 64), :] = kr
                ktiles[t] = (ku, kr)
                if t >= 1:
                    lo = iota(I32, (64,128), 1) < 64
                    ku0, kr0 = ktiles.pop(t-1)
                    kw_ref[2*t-1, pl.ds(i*64, 64), :] = jnp.where(lo, kr0, kr)
                    ks_ref[2*t-1, pl.ds(i*64, 64), :] = jnp.where(lo, ku, ku0)
            return f
        def qvpiece(r):
            def f():
                o = nt_dot(wT_ref[r*128:(r+1)*128, :], x_ref[rows, :])
                if r < 5:
                    qT_ref[i, pl.ds(r*64, 64), :] = bc((o * QSCALE).astype(BF), U32)
                else:
                    vT_ref[i, pl.ds((r-5)*64, 64), :] = bc(o.astype(BF), U32)
            return f
        return [kpiece(t) for t in range(5)], [qvpiece(r) for r in range(10)]

    def qwin(i, h):
        c0, base, a, off = head_geom(h)
        q0 = qT_ref[i, a//2:a//2+8, :]; q1 = qT_ref[i, a//2+8:a//2+16, :]
        o2 = off//2
        q0 = jnp.where(sub8 >= o2, q0, zero8)
        q1 = jnp.where(sub8 < o2 + 2, q1, zero8)
        return q0, q1, (a - base)//16
    def W_from(parts):
        return bc(jnp.concatenate([parts.get(j, zero8) for j in range(8)], axis=0), BF)
    def lanemask(h):
        c0, base, a, off = head_geom(h)
        A = c0 - base
        if A + DH <= 64: return lane8 < 64
        if A >= 64: return lane8 >= 64
        return (lane8 >= 32) & (lane8 < 96)
    def qk(i, h):
        c0, base, a, off = head_geom(h)
        w = base // 64
        q0, q1, p = qwin(i, h)
        d = sub8 - lane8
        def kblk(ref, j, r0, n): return ref[w, pl.ds(j*64 + r0, n), :]
        res = []
        W1 = None
        if i != 2 or True:
            W1 = W_from({p: q0, p+1: q1})
        if i >= 1:
            res.append(dot(bc(kblk(kw_ref, i-1, 0, 64), BF), W1))
        if i >= 2:
            lo = lane8 < 64
            W2 = W_from({p: jnp.where(lo, q0, zero8), p+1: jnp.where(lo, q1, zero8),
                         (p+4) % 8: jnp.where(lo, zero8, q0), (p+5) % 8: jnp.where(lo, zero8, q1)})
            lm = lanemask(h)
            l12 = [jnp.where(lm, kblk(kw_ref, i-2, j*8, 8), kblk(ks_ref, i, j*8, 8)) for j in range(8)]
            l3 = [jnp.where(lm, kblk(kw_ref, i, j*8, 8), kblk(ks_ref, i-2, 32 + j*8, 8)) for j in range(4)]
            s = dot(bc(jnp.concatenate(l12 + l3, axis=0), BF), W2)
            mg = []
            for j in range(8):
                cond = (d + 8*j > 0) | (lane8 >= 64)
                mg.append(jnp.where(cond, s[8*j:8*j+8], s[128+8*j:128+8*j+8]))
            for j in range(8, 16):
                cond = (d + 8*j > 0) & (lane8 >= 64)
                mg.append(jnp.where(cond, s[128+8*(j-8):128+8*(j-8)+8], s[8*j:8*j+8]))
            res.append(jnp.concatenate(mg, axis=0))
        else:
            s = dot(bc(kblk(kw_ref, i, 0, 64), BF), W1)
            mg = [jnp.where(d + 8*j > 0, NEG, s[8*j:8*j+8]) for j in range(16)]
            res.append(jnp.concatenate(mg, axis=0))
        return res
    def softmax(ss):
        m = ss[0]
        for s in ss[1:]: m = jnp.maximum(m, s)
        m = jnp.max(m, axis=0, keepdims=True)
        return [jnp.exp2(s - m).astype(BF) for s in ss]
    ones8 = jnp.full((8,128), 0x3F803F80, U32)
    def pv(i, h, ps):
        c0, base, a, off = head_geom(h)
        ones_lo = off >= 8
        if i >= 2:
            pm = bc(ps[1], U32)
            pn = pm & mk_ref[...]
            po = pm ^ pn
            pl_ = [(i-2, bc(po, BF)), (i-1, ps[0]), (i, bc(pn, BF))]
        elif i == 1:
            pl_ = [(0, ps[0]), (1, ps[1])]
        else:
            pl_ = [(0, ps[0])]
        acc = None
        for j, p in pl_:
            v0 = vT_ref[j, a//2:a//2+8, :]; v1 = vT_ref[j, a//2+8:a//2+16, :]
            if ones_lo: v0 = jnp.where(sub8 < 4, ones8, v0)
            else: v1 = jnp.where(sub8 >= 4, ones8, v1)
            o = dot(bc(jnp.concatenate([v0, v1], axis=0), BF), p)
            acc = o if acc is None else acc + o
        l = acc[0:8] if ones_lo else acc[24:32]
        inv = 1.0 / l
        return acc, inv
    def pv_pair(i, h0, ps0, ps1):
        res = {}
        for h, ps in ((h0, ps0), (h0+1, ps1)):
            c0, base, a, off = head_geom(h)
            acc, inv = pv(i, h, ps)
            for m in range(c0 // 8, (c0 + DH + 7) // 8):
                v = acc[8*m - a: 8*m - a + 8] * inv
                if m in res: res[m] = jnp.where(sub8 < 4, res[m], v)
                else: res[m] = v
        for m, v in res.items():
            oT_ref[i % 2, pl.ds(8*m, 8), :] = v
    def att_pieces(i):
        groups = [list(range(g, g+G)) for g in range(0, H, G)]
        n = len(groups)
        st_s = {}; st_p = {}
        def step(gi):
            def f():
                if gi < n: st_s[gi] = [qk(i, h) for h in groups[gi]]
                if 0 <= gi - 2 < n:
                    pss = st_p.pop(gi-2); hs = groups[gi-2]
                    for j in range(0, G, 2): pv_pair(i, hs[j], pss[j], pss[j+1])
                if 0 <= gi - 1 < n: st_p[gi-1] = [softmax(ss) for ss in st_s.pop(gi-1)]
            return f
        return [step(gi) for gi in range(n + 2)]

    def out_pieces(i):
        ot = {}
        def npiece(t):
            def f():
                if t == 0:
                    for u in range(5):
                        ot[u] = oT_ref[i % 2, pl.ds(u*128, 128), :].astype(BF).T
                o = jnp.concatenate([ot[u] for u in range(5)], axis=1)
                y_ref[pl.ds(i*128, 128), t*128:(t+1)*128] = dot(o, wo_ref[:, t*128:(t+1)*128]).astype(BF)
                if t == 4:
                    c = mk_copy(y_ref.at[pl.ds(i*128, 128), :], o_hbm.at[pl.ds(i*128, 128), pl.ds(D, D)])
                    c.start(); out_copies.append(c)
            return f
        return [npiece(t) for t in range(5)]

    A = AParts(xa_ref, wr_ref, wi_ref, M_ref, N_ref, Gf_ref, Gi_ref, gi_ref, Wp_ref, Sf_ref, Yb_ref, Rb_ref, ya_ref, srcs, a_out_dma)
    for c in (cp_w[0], cp_x[0], cp_w[1], cp_x[1], cp_w[2], cp_cst, cp_x[2]): c.start()
    cp_w[0].wait(); cp_x[0].wait()
    k0, qv0 = proj_pieces(0); k1_, qv1 = proj_pieces(1)
    for f in k0: f()
    for f in k1_: f()
    cp_w[1].wait()
    for c in (cp_wo, cp_x[3], cp_M, cp_xa): c.start()
    for r in range(5):
        for c in range(5):
            wT_ref[c*128:(c+1)*128, r*128:(r+1)*128] = wqkv_ref[r*128:(r+1)*128, c*128:(c+1)*128].T
    for f in qv0[:5]: f()
    cp_w[2].wait()
    for c in (cp_wr, cp_wi, cp_Gf, cp_Gi, cp_N): c.start()
    for r in range(5):
        for c in range(5):
            wT_ref[640 + c*128:640 + (c+1)*128, r*128:(r+1)*128] = wqkv_ref[r*128:(r+1)*128, 1280 + c*128:1280 + (c+1)*128].T
    for f in qv0[5:]: f()
    cp_cst.wait(); cp_x[1].wait()
    def waiter(*cs):
        def f():
            for c in cs: c.wait()
        return f
    a_f1 = [waiter(cp_M, cp_xa)] + A.f1_pieces()
    a_wp = [waiter(cp_wr, cp_wi)] + A.wprep_pieces()
    a_f2 = A.f2_pieces()
    a_m = [waiter(cp_Gf, cp_Gi)] + A.m_pieces()
    a_i2 = A.i2_pieces()
    a_i1 = [waiter(cp_N)] + A.i1_pieces()
    def split(lst, n):
        k = len(lst); return [lst[(j*k)//n:((j+1)*k)//n] for j in range(n)]
    a_plan = {s: [] for s in range(NB + 2)}
    def put(lst, slots):
        for s_, part in zip(slots, split(lst, len(slots))):
            if part: a_plan[s_].append(part)
    P = plan or dict(f1=(2,3,4,5), wp=(3,4,5), f2=(6,), m=(7,8,9,10), i2=(11,), i1=(12,13,14,15))
    put(a_f1, P["f1"]); put(a_wp, P["wp"]); put(a_f2, P["f2"]); put(a_m, P["m"]); put(a_i2, P["i2"]); put(a_i1, P["i1"])
    waited = {0, 1}
    for i in range(NB + 1):
        streams = []
        if i < NB: streams.append(att_pieces(i))
        if i + 1 < NB:
            ch = x_chunk_of_block[i+1]
            if ch not in waited:
                cp_x[ch].wait(); waited.add(ch)
            if i == 0: streams.append(qv1)
            else:
                kk, qq = proj_pieces(i+1); streams.append(kk + qq)
        if i == 1: cp_wo.wait()
        if i >= 1: streams.append(out_pieces(i-1))
        streams += a_plan[i]
        merge_streams(streams)
    for c in out_copies: c.wait()

def make_full(**kw):
    M, N, Gf, Gi, gi8, srcs = a_consts()
    cst = np.concatenate([new_mask_const(), gi8.view(np.uint32)], axis=0)
    def f(A_x, A_w_r, A_w_i, B_x, B_wqkv, B_wo):
        anyspec = pl.BlockSpec(memory_space=pltpu.HBM)
        out = pl.pallas_call(
            functools.partial(full_kernel, srcs=srcs, **kw),
            out_shape=jax.ShapeDtypeStruct((S, 2*D), BF),
            in_specs=[anyspec]*11, out_specs=anyspec,
            scratch_shapes=[pltpu.VMEM((S, D), BF), pltpu.VMEM((321, S), BF), pltpu.VMEM((321, S), BF),
                            pltpu.VMEM((640, 256), BF), pltpu.VMEM((768, 256), BF),
                            pltpu.VMEM((32,128,128), BF), pltpu.VMEM((32,128,128), BF),
                            pltpu.VMEM((2, 3, 17*64, 128), U32),
                            pltpu.VMEM((3, 2, 4, 8, 64, 128), F32),
                            pltpu.VMEM((32, 3, 128, 128), BF),
                            pltpu.VMEM((6, S, 128), BF),
                            pltpu.VMEM((S, D), BF),
                            pltpu.VMEM((S, D), BF), pltpu.VMEM((D, 3*D), BF), pltpu.VMEM((D, D), BF), pltpu.VMEM((72,128), U32),
                            pltpu.VMEM((1280, 640), BF),
                            pltpu.VMEM((NB, 320, 128), U32), pltpu.VMEM((NB, 320, 128), U32),
                            pltpu.VMEM((9, S//2, 128), U32), pltpu.VMEM((9, S//2, 128), U32),
                            pltpu.VMEM((2, 640, 128), F32), pltpu.VMEM((S, D), BF),
                            pltpu.SemaphoreType.DMA((16 + 2*NB,))],
            compiler_params=pltpu.CompilerParams(vmem_limit_bytes=110*2**20), name="fk")(
                A_x.reshape(S, D), A_w_r.T, A_w_i.T, B_x.reshape(S, D), B_wqkv, B_wo, cst, M, N, Gf, Gi)
        return out.reshape(1, S, 2*D)
    return f


_KERNEL_FN = make_full()


@jax.jit
def pallas_concat_heads__spectral_gfnet__sliding_block__prompt_kernel(
    A_x: jax.Array,
    A_w_r: jax.Array,
    A_w_i: jax.Array,
    B_x: jax.Array,
    B_wqkv: jax.Array,
    B_wo: jax.Array,
):
    return _KERNEL_FN(A_x, A_w_r, A_w_i, B_x, B_wqkv, B_wo)
```

```python
import contextlib
import functools
import itertools

import jax
import jax.numpy as jnp
import numpy as np
from jax.experimental import pallas as pl
from jax.experimental.pallas import tpu as pltpu

BF = jnp.bfloat16
F32 = jnp.float32
U32 = jnp.uint32
I32 = jnp.int32
iota = jax.lax.broadcasted_iota


dot = functools.partial(jnp.dot, preferred_element_type=F32)
nt_dot = functools.partial(jax.lax.dot_general, dimension_numbers=(((1,), (1,)), ((), ())), preferred_element_type=F32)


def bc(x, dt):
    return pltpu.bitcast(x, dt)

S, D = 2048, 640
C1, C2 = np.cos(2*np.pi/5), np.cos(4*np.pi/5)
S1, S2 = np.sin(2*np.pi/5), np.sin(4*np.pi/5)
RHO = S2 / S1

def lane_layout():
    cls = [((0,1),38), ((0,2),13), ((1,0),38), ((1,2),13), ((2,0),13), ((2,1),13)]
    a_src = []; b_src = []
    for (a, b), n in cls:
        a_src += [a]*n; b_src += [b]*n
    a_src = np.array(a_src); b_src = np.array(b_src)
    c_src = np.full(128, -1)
    for l in range(128):
        a, b = a_src[l], b_src[l]
        if {a, b} == {1, 2}: c_src[l] = 0
        elif {a, b} == {0, 2}: c_src[l] = 1
    c_src[:13] = 2
    ks = np.arange(321)
    def assign(src, res):
        out = np.full(128, -1)
        for s in range(3):
            cand = [k for k in ks if k // 128 == s and (k % 5) in res]
            lanes = np.nonzero(src == s)[0]
            assert len(cand) == len(lanes), (s, len(cand), len(lanes))
            out[lanes] = cand
        return out
    kA = assign(a_src, (1, 4)); kB = assign(b_src, (2, 3)); kC = assign(c_src, (0,))
    gidx = np.zeros((3, 128), np.int32)
    for kk, src in ((kA, a_src), (kB, b_src), (kC, c_src)):
        for l in range(128):
            if kk[l] >= 0:
                gidx[src[l], l] = kk[l] - 128*src[l]
    return kA, kB, kC, a_src, b_src, c_src, gidx

def row_mats():
    kA, kB, kC, *_ = lane_layout()
    m2 = np.arange(128)[:, None]
    def cs(k):
        ang = 2*np.pi*m2*np.where(k >= 0, k, 0)[None, :]/D
        v = (k >= 0)[None, :]
        return np.cos(ang)*v, np.sin(ang)*v
    def fwd_pair(k, first):
        C, Sn = cs(k)
        sg = np.where(k % 5 == first, -1.0, 1.0)[None, :] * S1
        M = np.zeros((256, 256))
        M[:128, :128] = C; M[:128, 128:] = -Sn
        M[128:, :128] = sg*Sn; M[128:, 128:] = sg*C
        return M
    MA = fwd_pair(kA, 1); MB = fwd_pair(kB, 2)
    C, Sn = cs(kC)
    MC = np.concatenate([C, -Sn], axis=1)
    norm = 1.0/(S*D)
    def inv_pair(k, first):
        C, Sn = cs(k)
        w = 2.0*norm
        sg = np.where(k % 5 == first, 1.0, -1.0)[None, :] * S1
        N = np.zeros((256, 256))
        N[:128, :128] = (w*C).T; N[128:, :128] = (-w*Sn).T
        N[:128, 128:] = (w*sg*Sn).T; N[128:, 128:] = (w*sg*C).T
        return N
    NA = inv_pair(kA, 1); NB = inv_pair(kB, 2)
    w = np.where((kC == 0) | (kC == 320), 1.0, 2.0)[None, :]*norm
    NC = np.concatenate([(w*C).T, (-w*Sn).T], axis=0)
    return MA, MB, MC, NA, NB, NC

def col_mats():
    k2 = np.arange(64)[:, None]; n2 = np.arange(64)[None, :]
    Gf = np.zeros((32, 128, 128))
    for k1 in range(32):
        ang = -2*np.pi*((n2*(k1 + 32*k2)) % S)/S
        gr, gi = np.cos(ang), np.sin(ang)
        Gf[k1, :64, :64] = gr; Gf[k1, :64, 64:] = -gi
        Gf[k1, 64:, :64] = gi; Gf[k1, 64:, 64:] = gr
    Gi = Gf.transpose(0, 2, 1).copy()
    return Gf, Gi


RT = float(np.sqrt(0.5)); R54 = float(np.sqrt(5)/4); RHO = float(RHO)
def cmul_const(z, ang_num, ang_den, sign):
    x, y = z
    n = (ang_num * 8) % (8*ang_den)
    if ang_num % ang_den == 0: return z
    if (ang_num * 4) % ang_den == 0:
        q = ((ang_num * 4) // ang_den) % 4
        q = q if sign > 0 else (-q) % 4
        if q == 1: return (-y, x)
        if q == 2: return (-x, -y)
        if q == 3: return (y, -x)
    if (ang_num * 8) % ang_den == 0:
        o = ((ang_num * 8) // ang_den) % 8
        o = o if sign > 0 else (-o) % 8
        c = 1 if o in (1, 7) else -1
        d = 1 if o in (1, 3) else -1
        if c == 1 and d == 1: return ((x - y) * RT, (x + y) * RT)
        if c == 1 and d == -1: return ((x + y) * RT, (y - x) * RT)
        if c == -1 and d == 1: return ((x + y) * (-RT), (x - y) * RT)
        return ((y - x) * RT, (x + y) * (-RT))
    ang = sign * 2*np.pi*ang_num/ang_den
    c, d = float(np.cos(ang)), float(np.sin(ang))
    return (x*c - y*d, x*d + y*c)

def cadd(a, b): return (a[0]+b[0], a[1]+b[1])
def csub(a, b): return (a[0]-b[0], a[1]-b[1])
def rot(t, u, sign):
    if sign > 0:
        return (t[0]-u[1], t[1]+u[0]), (t[0]+u[1], t[1]-u[0])
    return (t[0]+u[1], t[1]-u[0]), (t[0]-u[1], t[1]+u[0])

def radix4(z, sign):
    t0, t1, t2, t3 = cadd(z[0], z[2]), csub(z[0], z[2]), cadd(z[1], z[3]), csub(z[1], z[3])
    s1, s3 = rot(t1, t3, sign)
    return [cadd(t0, t2), s1, csub(t0, t2), s3]

def radix8(z, sign):
    u = [cadd(z[b], z[b+4]) for b in range(4)]
    v = [csub(z[b], z[b+4]) for b in range(4)]
    ev = radix4(u, sign)
    v1 = cmul_const(v[1], 1, 8, sign); v3 = cmul_const(v[3], 3, 8, sign)
    t0, t1 = rot(v[0], v[2], sign)
    t2, t3 = cadd(v1, v3), csub(v1, v3)
    s1, s3 = rot(t1, t3, sign)
    od = [cadd(t0, t2), s1, csub(t0, t2), s3]
    out = []
    for j in range(4): out += [ev[j], od[j]]
    return out

def lane_sel_mask(src, s, lane8):
    m = None; l = 0
    while l < 128:
        if src[l] == s:
            r = l
            while r < 128 and src[r] == s: r += 1
            t = (lane8 >= l) & (lane8 < r)
            m = t if m is None else (m | t)
            l = r
        else: l += 1
    return m


H, DH, WIN = 32, 20, 256
NB = S // 128
NEG = -1e30
QSCALE = float((DH ** -0.5) * np.log2(np.e))


def head_geom(h):
    c0 = DH*h; t = c0//128
    straddle = (c0+DH-1)//128 != t
    base = 128*t + (64 if straddle else 0)
    a = (c0//16)*16; off = c0 - a
    return c0, base, a, off


def merge_streams(streams):
    items = []
    for si, st in enumerate(streams):
        n = len(st)
        for j, f in enumerate(st):
            items.append(((j + 0.5) / n, si, j, f))
    items.sort(key=lambda t: (t[0], t[1]))
    for _, _, _, f in items:
        f()


def pack_rows(a):
    u = np.ascontiguousarray(a.astype(BF)).view(np.uint16).astype(np.uint32)
    return u[..., 0::2, :] | (u[..., 1::2, :] << np.uint32(16))


def a_consts():
    kA, kB, kC, a_src, b_src, c_src, gidx = lane_layout()
    MA, MB, MC, NA, NB_, NC = row_mats(); Gf, Gi = col_mats()
    M = pack_rows(np.concatenate([MA, MB, MC], 0))
    N = pack_rows(np.concatenate([NA, NB_, np.concatenate([NC, np.zeros((256, 128))], 1)], 0))
    gi8 = np.zeros((8, 128), np.int32); gi8[:3] = gidx
    return M, N, pack_rows(Gf), pack_rows(Gi), gi8, (a_src, b_src, c_src)


def full_kernel(xa_hbm, wr_hbm, wi_hbm, x_hbm, wqkv_hbm, wo_hbm, gi_hbm, M_hbm, N_hbm, Gf_hbm, Gi_hbm, o_hbm,
                xa_ref, wr_ref, wi_ref, M_ref, N_ref, Gf_ref, Gi_ref, Wp_ref, Sf_ref, Yb_ref, Rb_ref, ya_ref,
                xraw_ref, wraw_ref, woraw_ref,
                x_ref, wk_ref, wo_ref, gi_ref, wT_ref, qT_ref, vT_ref, kw_ref, ks_ref, oT_ref, y_ref, sems,
                *, srcs, G=4, plan=None, UF=2, scopes=0, order='fine', LAG=1, online=True, QB=32, MLAG=2, MSPLIT=False, qv_first=False, out_mode=0, QVN=1, OUTN=5, out_prep=False):
    a_src, b_src, c_src = srcs
    Tf_ref = Sf_ref
    x_u, wk_u, wo_u = x_ref, wk_ref, wo_ref
    qT_u, vT_u, kw_u, ks_u = (r.bitcast(U32) for r in (qT_ref, vT_ref, kw_ref, ks_ref))

    nsem = [0]
    def group(pairs):
        s = sems.at[nsem[0]]; nsem[0] += 1
        return [pltpu.make_async_copy(a, b, s) for a, b in pairs]
    def start(g):
        for c in g: c.start()
    def wait(g):
        for c in g: c.wait()
    def rows_in(src, dst, r0, n):
        return [(src.at[pl.ds(r0, n), :], dst.at[pl.ds(r0, n), :])]
    def cols_in(j):
        return [(wqkv_hbm.at[:, pl.ds(D*j, D)], wraw_ref.at[j])]
    xchunks = ((0, 128), (128, 256), (384, 512), (896, 512), (1408, 640))
    x_in = [rows_in(x_hbm, xraw_ref, r0, n) for r0, n in xchunks]
    g0 = group(x_in[0] + cols_in(1))
    g1 = group(x_in[1]); g2 = group(x_in[2]); g3 = group(x_in[3])
    g4 = group(cols_in(0) + cols_in(2))
    g5 = group(x_in[4] + [(wo_hbm, woraw_ref)])
    g6 = group([(M_hbm, M_ref), (xa_hbm, xa_ref)])
    g7 = group([(wr_hbm, wr_ref), (wi_hbm, wi_ref), (gi_hbm, gi_ref), (Gf_hbm, Gf_ref), (Gi_hbm, Gi_ref), (N_hbm, N_ref)])
    out_sem = sems.at[nsem[0]]; nsem[0] += 1
    out_copies = []
    def out_dma(src_ref, r0, n, col0):
        for t in range(5):
            c = pltpu.make_async_copy(src_ref.at[t, pl.ds(r0, n), :], o_hbm.at[pl.ds(r0, n), pl.ds(col0 + 128*t, 128)], out_sem)
            c.start(); out_copies.append(c)

    sub8 = iota(I32, (8, 128), 0); lane8 = iota(I32, (8, 128), 1)
    zero8 = jnp.zeros((8, 128), U32)

    def xrows(i):
        return jnp.concatenate([bc(x_u[t, pl.ds(i*64, 64), :], BF) for t in range(5)], axis=1)

    def proj_pieces(i):
        def kpiece(t):
            def f():
                kt = dot(xrows(i), bc(wk_u[t], BF))
                kw_ref[2*t, pl.ds(i*128, 128), :] = kt.astype(BF)
                ku = kw_u[2*t, pl.ds(i*64, 64), :]
                if QB == 64:
                    kr = pltpu.roll(ku, 64, 1)
                    ks_u[1, 2*t, pl.ds(i*64, 64), :] = kr
                    if t >= 1:
                        lo = iota(I32, (64, 128), 1) < 64
                        kw_u[2*t-1, pl.ds(i*64, 64), :] = jnp.where(lo, ks_u[1, 2*t-2, pl.ds(i*64, 64), :], kr)
                        ks_u[1, 2*t-1, pl.ds(i*64, 64), :] = jnp.where(lo, ku, kw_u[2*t-2, pl.ds(i*64, 64), :])
                else:
                    rot = [ku] + [pltpu.roll(ku, 32*j, 1) for j in (1, 2, 3)]
                    for j in (1, 2, 3): ks_u[j, 2*t, pl.ds(i*64, 64), :] = rot[j]
                    if t >= 1:
                        ln = iota(I32, (64, 128), 1)
                        for j in range(4):
                            jj = (j + 2) % 4
                            prev = kw_u[2*t-2, pl.ds(i*64, 64), :] if jj == 0 else ks_u[jj, 2*t-2, pl.ds(i*64, 64), :]
                            cond = ((ln >= 32*j) & (ln < 32*j + 64)) if j < 2 else ((ln >= 32*j) | (ln < 32*j - 64))
                            v = jnp.where(cond, prev, rot[jj])
                            if j == 0: kw_u[2*t-1, pl.ds(i*64, 64), :] = v
                            else: ks_u[j, 2*t-1, pl.ds(i*64, 64), :] = v
            return f
        def qvpiece(r, n):
            def f():
                o = nt_dot(wT_ref[r*128:(r+n)*128, :], xrows(i))
                for u in range(n):
                    ou = o[u*128:(u+1)*128]
                    if r + u < 5:
                        qT_ref[i, (r+u)*128:(r+u+1)*128, :] = (ou * QSCALE).astype(BF)
                    else:
                        vT_ref[i, (r+u-5)*128:(r+u-4)*128, :] = ou.astype(BF)
            return f
        return [kpiece(t) for t in range(5)], [qvpiece(r, QVN) for r in range(0, 10, QVN)]

    def qwin(i, h):
        c0, base, a, off = head_geom(h)
        q0 = qT_u[i, a//2:a//2+8, :]; q1 = qT_u[i, a//2+8:a//2+16, :]
        o2 = off//2
        q0 = jnp.where(sub8 >= o2, q0, zero8)
        q1 = jnp.where(sub8 < o2 + 2, q1, zero8)
        return q0, q1, (a - base)//16
    def W_from(parts):
        return bc(jnp.concatenate([parts.get(j, zero8) for j in range(8)], axis=0), BF)
    def lanemask(h):
        c0, base, a, off = head_geom(h)
        A = c0 - base
        if A + DH <= 64: return lane8 < 64
        if A >= 64: return lane8 >= 64
        return (lane8 >= 32) & (lane8 < 96)
    def qk(i, h):
        c0, base, a, off = head_geom(h)
        w = base // 64
        q0, q1, p = qwin(i, h)
        d = sub8 - lane8
        def kblk(ref, j, r0, n): return ref[w, pl.ds(j*64 + r0, n), :]
        res = []
        W1 = W_from({p: q0, p+1: q1})
        if i >= 1:
            res.append(dot(bc(kblk(kw_u, i-1, 0, 64), BF), W1))
        if i >= 2 and QB == 64:
            ks1 = ks_u.at[1]
            lo = lane8 < 64
            W2 = W_from({p: jnp.where(lo, q0, zero8), p+1: jnp.where(lo, q1, zero8),
                         (p+4) % 8: jnp.where(lo, zero8, q0), (p+5) % 8: jnp.where(lo, zero8, q1)})
            lm = lanemask(h)
            l12 = [jnp.where(lm, kblk(kw_u, i-2, j*8, 8), kblk(ks1, i, j*8, 8)) for j in range(8)]
            l3 = [jnp.where(lm, kblk(kw_u, i, j*8, 8), kblk(ks1, i-2, 32 + j*8, 8)) for j in range(4)]
            s = dot(bc(jnp.concatenate(l12 + l3, axis=0), BF), W2)
            mg = []
            for j in range(8):
                cond = (d + 8*j > 0) | (lane8 >= 64)
                mg.append(jnp.where(cond, s[8*j:8*j+8], s[128+8*j:128+8*j+8]))
            for j in range(8, 16):
                cond = (d + 8*j > 0) & (lane8 >= 64)
                mg.append(jnp.where(cond, s[128+8*(j-8):128+8*(j-8)+8], s[8*j:8*j+8]))
            res.append(jnp.concatenate(mg, axis=0))
        elif i >= 2:
            A0 = c0 - base - 6
            def inset(j):
                lo_, hi_ = (A0 + 32*j) % 128, (A0 + 32*j) % 128 + 32
                return ((lane8 >= lo_) & (lane8 < hi_)) if hi_ <= 128 else ((lane8 >= lo_) | (lane8 < hi_ - 128))
            msk = [inset(j) for j in range(3)]
            parts = {}
            for j in range(4):
                qm = (lane8 >= 32*j) & (lane8 < 32*j + 32)
                parts[(p + 2*j) % 8] = jnp.where(qm, q0, zero8)
                parts[(p + 2*j + 1) % 8] = jnp.where(qm, q1, zero8)
            W2 = W_from(parts)
            def krot(j, blk, r0):
                ref = kw_u if j == 0 else ks_u.at[j]
                return kblk(ref, blk, r0, 8)
            def compose(a):
                return jnp.where(msk[0], a[0], jnp.where(msk[1], a[1], jnp.where(msk[2], a[2], a[3])))
            la = [compose([krot(j, i-2 if j <= v // 2 else i, v*8) for j in range(4)]) for v in range(8)]
            lb = [compose([krot(j, i, 16*j + v*8) for j in range(4)]) for v in range(2)]
            s = dot(bc(jnp.concatenate(la + lb, axis=0), BF), W2)
            mg = []
            for v in range(16):
                ci = v // 4
                cond = (lane8 >= 32*ci) & (lane8 < 32*ci + 32) & (d + 8*v <= 0)
                mg.append(jnp.where(cond, s[128 + 8*(v % 4):128 + 8*(v % 4) + 8], s[8*v:8*v+8]))
            res.append(jnp.concatenate(mg, axis=0))
        else:
            s = dot(bc(kblk(kw_u, i, 0, 64), BF), W1)
            mg = [jnp.where(d + 8*j > 0, NEG, s[8*j:8*j+8]) for j in range(16)]
            res.append(jnp.concatenate(mg, axis=0))
        return res
    m_new = iota(I32, (128, 128), 0) <= iota(I32, (128, 128), 1)
    def softmax(i, ss):
        if online and len(ss) == 2:
            m1 = jnp.max(ss[0], axis=0, keepdims=True)
            p1 = jnp.exp2(ss[0] - m1).astype(BF)
            m2 = jnp.maximum(m1, jnp.max(ss[1], axis=0, keepdims=True))
            p2 = jnp.exp2(ss[1] - m2)
            alpha = jnp.exp2(m1 - m2)
            if i >= 2:
                return [(i-1, p1, alpha), (i-2, jnp.where(m_new, 0.0, p2).astype(BF), None), (i, jnp.where(m_new, p2, 0.0).astype(BF), None)]
            return [(0, p1, alpha), (1, p2.astype(BF), None)]
        m = ss[0]
        for s in ss[1:]: m = jnp.maximum(m, s)
        m = jnp.max(m, axis=0, keepdims=True)
        ps = [jnp.exp2(s - m) for s in ss]
        if i >= 2:
            return [(i-1, ps[0].astype(BF), None), (i-2, jnp.where(m_new, 0.0, ps[1]).astype(BF), None), (i, jnp.where(m_new, ps[1], 0.0).astype(BF), None)]
        if i == 1:
            return [(0, ps[0].astype(BF), None), (1, ps[1].astype(BF), None)]
        return [(0, ps[0].astype(BF), None)]
    ones8 = jnp.full((8, 128), 0x3F803F80, U32)
    def pv(i, h, pl_):
        c0, base, a, off = head_geom(h)
        ones_lo = off >= 8
        acc = None
        for j, p, alpha in pl_:
            v0 = vT_u[j, a//2:a//2+8, :]; v1 = vT_u[j, a//2+8:a//2+16, :]
            if ones_lo: v0 = jnp.where(sub8 < 4, ones8, v0)
            else: v1 = jnp.where(sub8 >= 4, ones8, v1)
            o = dot(bc(jnp.concatenate([v0, v1], axis=0), BF), p)
            if alpha is not None: o = o * alpha
            acc = o if acc is None else acc + o
        l = acc[0:8] if ones_lo else acc[24:32]
        r = pltpu.reciprocal(l, approx=True)
        inv = r * (2.0 - l * r)
        return acc, inv
    def pv_pair(i, h0, get_p):
        res = {}
        for h in (h0, h0+1):
            c0, base, a, off = head_geom(h)
            acc, inv = pv(i, h, get_p(h))
            for m in range(c0 // 8, (c0 + DH + 7) // 8):
                v = acc[8*m - a: 8*m - a + 8] * inv
                if m in res: res[m] = jnp.where(sub8 < 4, res[m], v)
                else: res[m] = v
        for m, v in res.items():
            oT_ref[i % 2, pl.ds(8*m, 8), :] = v
    def att_steps():
        units = [(i, list(range(g, g+G))) for i in range(NB) for g in range(0, H, G)]
        n = len(units)
        st_s = {}; st_p = {}
        def step(gi):
            def f():
                def do_qk():
                    if gi < n:
                        i, hs = units[gi]
                        st_s[gi] = {h: qk(i, h) for h in hs}
                def do_sm_pv():
                    if 0 <= gi - 1 < n:
                        i, hs = units[gi-1]
                        sss = st_s.pop(gi-1)
                        for j in range(0, G, 2): pv_pair(i, hs[j], lambda h: softmax(i, sss.pop(h)))
                if order == "pipe3":
                    do_qk()
                    if 0 <= gi - 2 < n:
                        i, hs = units[gi-2]
                        pss = st_p.pop(gi-2)
                        for j in range(0, G, 2): pv_pair(i, hs[j], lambda h: pss.pop(h))
                    if 0 <= gi - 1 < n:
                        i, hs = units[gi-1]
                        sss = st_s.pop(gi-1)
                        st_p[gi-1] = {h: softmax(i, sss[h]) for h in hs}
                elif order == "pipe2":
                    do_qk(); do_sm_pv()
                elif order == "pipe2r":
                    do_sm_pv(); do_qk()
                elif order == "lag":
                    if 0 <= gi - LAG < n:
                        i, hs = units[gi-LAG]
                        sss = st_s.pop(gi-LAG)
                        for j in range(0, G, 2): pv_pair(i, hs[j], lambda h: softmax(i, sss.pop(h)))
                    do_qk()
                elif order == "lag3":
                    if 0 <= gi - LAG - 1 < n:
                        i, hs = units[gi-LAG-1]
                        pss = st_p.pop(gi-LAG-1)
                        for j in range(0, G, 2): pv_pair(i, hs[j], lambda h: pss.pop(h))
                    if 0 <= gi - LAG < n:
                        i, hs = units[gi-LAG]
                        sss = st_s.pop(gi-LAG)
                        st_p[gi-LAG] = {h: softmax(i, sss[h]) for h in hs}
                    do_qk()
                elif order == "fine":
                    for j in range(0, G, 2):
                        if 0 <= gi - 1 < n:
                            i, hs = units[gi-1]
                            sss = st_s[gi-1]
                            pv_pair(i, hs[j], lambda h: softmax(i, sss.pop(h)))
                        if gi < n:
                            i, hs = units[gi]
                            st_s.setdefault(gi, {})
                            for h in hs[j:j+2]: st_s[gi][h] = qk(i, h)
            return f
        return [step(gi) for gi in range(n + LAG + 2)]

    def out_pieces(i):
        ot = {}
        def prep():
            for u in range(5):
                ot[u] = oT_ref[i % 2, pl.ds(u*128, 128), :].astype(BF).T
        def npiece(t, n):
            def f():
                if t == 0 and not out_prep: prep()
                o = jnp.concatenate([ot[u] for u in range(5)], axis=1)
                w = jnp.concatenate([wo_u[t+v] for v in range(n)], axis=1) if n > 1 else wo_u[t]
                y = dot(o, bc(w, BF))
                for v in range(n):
                    y_ref[t+v, pl.ds(i*128, 128), :] = y[:, v*128:(v+1)*128].astype(BF)
            return f
        return ([prep] if out_prep else []) + [npiece(t, min(OUTN, 5-t)) for t in range(0, 5, OUTN)]

    def wprep_pieces():
        def piece(j, arr):
            def f():
                ref = (wr_ref, wi_ref)[arr]
                gidx = [jnp.broadcast_to(gi_ref[t:t+1, :], (8, 128)) for t in range(3)]
                mA0, mA1 = lane_sel_mask(a_src, 0, lane8), lane_sel_mask(a_src, 1, lane8)
                mB0, mB1 = lane_sel_mask(b_src, 0, lane8), lane_sel_mask(b_src, 1, lane8)
                mC0, mC1 = lane_sel_mask(c_src, 0, lane8), lane_sel_mask(c_src, 1, lane8)
                cols = slice(128*j, 128*j+128)
                t2 = jnp.concatenate([ref[256:321, cols], jnp.zeros((63, 128), BF)], axis=0)
                tiles = [bc(ref[0:128, cols].T, U32), bc(ref[128:256, cols].T, U32), bc(t2.T, U32)]
                for v in range(8):
                    u = 8*j + v
                    g = [jnp.take_along_axis(tiles[t][8*v:8*v+8], gidx[t], axis=1) for t in range(3)]
                    pos = 17*(u//2) + 8*(u % 2)
                    Wp_ref[arr, 0, pos:pos+8, :] = jnp.where(mA0, g[0], jnp.where(mA1, g[1], g[2]))
                    Wp_ref[arr, 1, pos:pos+8, :] = jnp.where(mB0, g[0], jnp.where(mB1, g[1], g[2]))
                    Wp_ref[arr, 2, pos:pos+8, :] = jnp.where(mC0, g[0], jnp.where(mC1, g[1], g[2]))
            return f
        return [piece(j, arr) for j in range(16) for arr in range(2)]

    def f1_pieces(UF):
        nr = 16*UF
        def piece(b, g):
            def f():
                def xt(t):
                    return jnp.concatenate([xa_ref[pl.ds(64*(8*a+b) + nr*g, nr), t*128:(t+1)*128] for a in range(4)], axis=0).astype(F32)
                T = [xt(t) for t in range(5)]
                p, q, r, w = T[1]+T[4], T[2]+T[3], T[1]-T[4], T[2]-T[3]
                u = p+q
                U0 = (T[0]+u).astype(BF)
                t1 = T[0] - 0.25*u; t2 = (p-q)*R54
                a1 = (t1+t2).astype(BF); a2 = (t1-t2).astype(BF)
                b1 = (r + RHO*w).astype(BF); b2 = (RHO*r - w).astype(BF)
                RA = dot(jnp.concatenate([a1, b1], axis=1), bc(M_ref[0:128, :], BF))
                RB = dot(jnp.concatenate([a2, b2], axis=1), bc(M_ref[128:256, :], BF))
                RC = dot(U0, bc(M_ref[256:320, :], BF))
                for P, R in enumerate((RA, RB, RC)):
                    z = [(R[nr*a:nr*a+nr, 0:128], R[nr*a:nr*a+nr, 128:256]) for a in range(4)]
                    Sx = radix4(z, -1)
                    for ka in range(4):
                        x, y = cmul_const(Sx[ka], b*ka, 32, -1)
                        Sf_ref[P, 0, ka, b, nr*g:nr*g+nr, :] = x
                        Sf_ref[P, 1, ka, b, nr*g:nr*g+nr, :] = y
            return f
        return [piece(b, g) for g in range(4//UF) for b in range(8)]

    def f2_pieces():
        def piece(ka, g, P):
            def f():
                z = [(Sf_ref[P, 0, ka, b, 16*g:16*g+16, :], Sf_ref[P, 1, ka, b, 16*g:16*g+16, :]) for b in range(8)]
                o = radix8(z, -1)
                for kb in range(8):
                    k1 = ka + 4*kb
                    Yb_ref[k1, P, 16*g:16*g+16, :] = o[kb][0].astype(BF)
                    Yb_ref[k1, P, 64+16*g:64+16*g+16, :] = o[kb][1].astype(BF)
            return f
        return [piece(ka, g, P) for ka in range(4) for P in range(3) for g in range(4)]

    def m_pieces():
        def m1(be, P, als):
            def f():
                for al in als:
                    k1 = be + 8*al
                    X = dot(bc(Gf_ref[k1], BF), Yb_ref[k1, P])
                    wr = Wp_ref[0, P, pl.ds(k1//2, 64, stride=17), :]
                    wi = Wp_ref[1, P, pl.ds(k1//2, 64, stride=17), :]
                    if k1 % 2 == 0:
                        wr = bc(wr << 16, F32); wi = bc(wi << 16, F32)
                    else:
                        wr = bc(wr & jnp.uint32(0xFFFF0000), F32); wi = bc(wi & jnp.uint32(0xFFFF0000), F32)
                    xr, xi = X[0:64], X[64:128]
                    Yb_ref[k1, P, 0:64, :] = (xr*wr - xi*wi).astype(BF)
                    Yb_ref[k1, P, 64:128, :] = (xr*wi + xi*wr).astype(BF)
            return f
        def m2(be, P):
            def f():
                V = []
                for al in range(4):
                    k1 = be + 8*al
                    Vv = dot(bc(Gi_ref[k1], BF), Yb_ref[k1, P])
                    V.append((Vv[0:64], Vv[64:128]))
                Tn = radix4(V, +1)
                for na in range(4):
                    x, y = cmul_const(Tn[na], be*na, 32, +1)
                    Tf_ref[P, 0, na, be] = x
                    Tf_ref[P, 1, na, be] = y
            return f
        units = [(be, P) for P in range(3) for be in range(8)]
        out = []
        for n_ in range(len(units) + MLAG):
            if n_ < len(units):
                if MSPLIT: out += [m1(*units[n_], (0, 1)), m1(*units[n_], (2, 3))]
                else: out.append(m1(*units[n_], (0, 1, 2, 3)))
            if n_ - MLAG >= 0: out.append(m2(*units[n_-MLAG]))
        return out

    def i2_pieces():
        def piece(na, g, P):
            def f():
                z = [(Tf_ref[P, 0, na, be, 16*g:16*g+16, :], Tf_ref[P, 1, na, be, 16*g:16*g+16, :]) for be in range(8)]
                o = radix8(z, +1)
                for nb in range(8):
                    n1 = na + 4*nb
                    Rb_ref[2*P, 64*n1+16*g:64*n1+16*g+16, :] = o[nb][0].astype(BF)
                    Rb_ref[2*P+1, 64*n1+16*g:64*n1+16*g+16, :] = o[nb][1].astype(BF)
            return f
        return [piece(na, g, P) for P in range(3) for na in range(4) for g in range(4)]

    def i1_pieces(R=128):
        def piece(j):
            def f():
                rows = slice(R*j, R*(j+1))
                EA = dot(jnp.concatenate([Rb_ref[0, rows, :], Rb_ref[1, rows, :]], axis=1), bc(N_ref[0:128, :], BF))
                EB = dot(jnp.concatenate([Rb_ref[2, rows, :], Rb_ref[3, rows, :]], axis=1), bc(N_ref[128:256, :], BF))
                U0 = dot(jnp.concatenate([Rb_ref[4, rows, :], Rb_ref[5, rows, :]], axis=1), bc(N_ref[256:384, 0:128], BF))
                e1, f1, e2, f2 = EA[:, :128], EA[:, 128:], EB[:, :128], EB[:, 128:]
                u = e1+e2
                t1 = U0 - 0.25*u; t2 = (e1-e2)*R54
                al, be = t1+t2, t1-t2
                ga = f1 + RHO*f2; de = RHO*f1 - f2
                ys = [U0+u, al-ga, be-de, be+de, al+ga]
                for t in range(5):
                    ya_ref[t, rows, :] = ys[t].astype(BF)
            return f
        return [piece(j) for j in range(S // R)]

    for g in (g0, g1, g2, g3, g4, g5, g6, g7): start(g)
    def retile(src, dst, r0, n):
        for t in range(5):
            dst[t, pl.ds(r0//2, n//2), :] = bc(src[pl.ds(r0, n), t*128:(t+1)*128], U32)
    def transposes(j, r0):
        for r in range(5):
            for c in range(5):
                wT_ref[r0 + c*128:r0 + (c+1)*128, r*128:(r+1)*128] = wraw_ref[j, r*128:(r+1)*128, c*128:(c+1)*128].T
    def kblocks(i0, i1):
        for i in range(i0, i1):
            retile(xraw_ref, x_ref, 128*i, 128)
            for f in proj_pieces(i)[0]: f()
    def scope(name):
        return jax.named_scope(name) if scopes else contextlib.nullcontext()
    with scope("p0w"): wait(g0)
    with scope("p0"):
        retile(wraw_ref.at[1], wk_ref, 0, D)
        kblocks(0, 1)
    with scope("p1w"): wait(g1)
    with scope("p1"): kblocks(1, 3)
    with scope("p2w"): wait(g2)
    with scope("p2"): kblocks(3, 7)
    with scope("p3w"): wait(g3)
    with scope("p3"): kblocks(7, 9)
    with scope("p4w"): wait(g4)
    with scope("p4"):
        transposes(0, 0); kblocks(9, 10); transposes(2, 640); kblocks(10, 11)
        for f in proj_pieces(0)[1]: f()
    with scope("p5w"): wait(g5)
    with scope("p5"):
        retile(woraw_ref, wo_ref, 0, D)
        kblocks(11, 16)

    GPB = H // G
    items = []
    def place(lst, lo, hi, prio):
        n = len(lst)
        for j, fn in enumerate(lst):
            items.append((lo + (hi - lo) * (j + 0.5) / n, prio, len(items), fn))
    def at(key, fn): items.append((key, -1, len(items), fn))
    for gi, fn in enumerate(att_steps()):
        items.append((gi + 0.5, 0, len(items), fn))
    if qv_first:
        for i in range(1, NB):
            for f in proj_pieces(i)[1]: f()
    else:
        for i in range(1, NB):
            place(proj_pieces(i)[1], GPB*(i-1), GPB*i + 0.4, 1)
    for i in range(NB):
        if out_mode == 0:
            place(out_pieces(i), GPB*(i+1) + LAG + 1, GPB*(i+2) + LAG + 1 if i < NB-1 else GPB*(i+1) + LAG + 2, 2)
        elif out_mode == 1:
            place(out_pieces(i), GPB*(i+1) + 2, GPB*(i+1) + 2.01, 2)
    P_ = plan or dict(f1=(2, 5), wp=(5.4, 6.6), f2=(5, 6), m=(6.6, 10.5), i2=(10.5, 11.5), i1=(11.5, 14.2))
    for name, lst in (("f1", f1_pieces(UF)), ("wp", wprep_pieces()), ("f2", f2_pieces()), ("m", m_pieces()), ("i2", i2_pieces()), ("i1", i1_pieces())):
        lo, hi = P_[name]
        place(lst, GPB*lo, GPB*hi, 3 if name != "wp" else 4)
    def sync(waits=(), outs=(), starts=()):
        def f():
            for g in starts: start(g)
            for g in waits: wait(g)
            for o in outs: out_dma(*o)
        return f
    at(GPB*2 - 0.01, sync(waits=(g6,)))
    at(GPB*5 + LAG + 1.01, sync(waits=(g7,), outs=((y_ref, 0, 384, D),)))
    at(GPB*14 + LAG + 1.01, sync(outs=((y_ref, 384, 1280, D), (ya_ref, 0, S, 0))))
    at(GPB*18, sync(outs=((y_ref, 1664, 384, D),)))
    items.sort(key=lambda t: t[:3])
    if scopes:
        for sl, grp in itertools.groupby(items, key=lambda t: int(t[0] // (GPB*scopes))):
            with jax.named_scope("slot%02d" % sl):
                for it in grp: it[3]()
    else:
        for it in items: it[3]()
    with scope("zztail"):
        for c in out_copies: c.wait()
    assert nsem[0] <= NSEM


NSEM = 9


def make_full(**kw):
    M, N, Gf, Gi, gi8, srcs = a_consts()
    def V(shape, dt): return pltpu.VMEM(shape, dt)
    def f(A_x, A_w_r, A_w_i, B_x, B_wqkv, B_wo):
        hbm = pl.BlockSpec(memory_space=pltpu.HBM)
        out = pl.pallas_call(
            functools.partial(full_kernel, srcs=srcs, **kw),
            out_shape=jax.ShapeDtypeStruct((S, 2*D), BF),
            in_specs=[hbm]*11, out_specs=hbm,
            scratch_shapes=[V((S, D), BF), V((321, S), BF), V((321, S), BF),
                            V((320, 256), U32), V((384, 256), U32),
                            V((32, 64, 128), U32), V((32, 64, 128), U32),
                            V((2, 3, 17*64, 128), U32),
                            V((3, 2, 4, 8, 64, 128), F32),
                            V((32, 3, 128, 128), BF),
                            V((6, S, 128), BF),
                            V((5, S, 128), BF),
                            V((S, D), BF), V((3, D, D), BF), V((D, D), BF),
                            V((5, S//2, 128), U32), V((5, D//2, 128), U32), V((5, D//2, 128), U32), V((8, 128), I32),
                            V((1280, 640), BF),
                            V((NB, 640, 128), BF), V((NB, 640, 128), BF),
                            V((9, S, 128), BF), V((4, 9, S, 128), BF),
                            V((2, 640, 128), F32), V((5, S, 128), BF),
                            pltpu.SemaphoreType.DMA((NSEM,))],
            compiler_params=pltpu.CompilerParams(vmem_limit_bytes=110*2**20), name="fk")(
                A_x.reshape(S, D), A_w_r.T, A_w_i.T, B_x.reshape(S, D), B_wqkv, B_wo, gi8, M, N, Gf, Gi)
        return out.reshape(1, S, 2*D)
    return f


_KERNEL_FN = make_full()


@jax.jit
def pallas_concat_heads__spectral_gfnet__sliding_block__prompt_kernel(
    A_x: jax.Array,
    A_w_r: jax.Array,
    A_w_i: jax.Array,
    B_x: jax.Array,
    B_wqkv: jax.Array,
    B_wo: jax.Array,
):
    return _KERNEL_FN(A_x, A_w_r, A_w_i, B_x, B_wqkv, B_wo)
```

```python
import contextlib
import functools
import itertools

import jax
import jax.numpy as jnp
import numpy as np
from jax.experimental import pallas as pl
from jax.experimental.pallas import tpu as pltpu

BF = jnp.bfloat16
F32 = jnp.float32
U32 = jnp.uint32
I32 = jnp.int32
iota = jax.lax.broadcasted_iota


dot = functools.partial(jnp.dot, preferred_element_type=F32)
nt_dot = functools.partial(jax.lax.dot_general, dimension_numbers=(((1,), (1,)), ((), ())), preferred_element_type=F32)


def bc(x, dt):
    return pltpu.bitcast(x, dt)

S, D = 2048, 640
C1, C2 = np.cos(2*np.pi/5), np.cos(4*np.pi/5)
S1, S2 = np.sin(2*np.pi/5), np.sin(4*np.pi/5)
RHO = S2 / S1

def lane_layout():
    cls = [((1, 2), 13), ((2, 1), 13), ((0, 2), 13), ((2, 0), 13), ((0, 1), 38), ((1, 0), 38)]
    a_src = []; b_src = []
    for (a, b), n in cls:
        a_src += [a]*n; b_src += [b]*n
    a_src = np.array(a_src); b_src = np.array(b_src)
    c_src = np.full(128, -1)
    c_src[0:26] = 0; c_src[26:52] = 1; c_src[52:65] = 2
    ks = np.arange(321)
    def assign(src, res):
        out = np.full(128, -1)
        for s in range(3):
            cand = [k for k in ks if k // 128 == s and (k % 5) in res]
            lanes = np.nonzero(src == s)[0]
            assert len(cand) == len(lanes), (s, len(cand), len(lanes))
            out[lanes] = cand
        return out
    kA = assign(a_src, (1, 4)); kB = assign(b_src, (2, 3)); kC = assign(c_src, (0,))
    assert kC[0] == 0 and kC[64] == 320
    gidx = np.zeros((3, 128), np.int32)
    used = np.zeros((3, 128), bool)
    for kk, src in ((kA, a_src), (kB, b_src), (kC, c_src)):
        for l in range(128):
            if kk[l] >= 0:
                assert not used[src[l], l]
                used[src[l], l] = True
                gidx[src[l], l] = kk[l] - 128*src[l]
    return kA, kB, kC, a_src, b_src, c_src, gidx


def row_mats():
    kA, kB, kC, *_ = lane_layout()
    m2 = np.arange(128)[:, None]
    def cs(k):
        ang = 2*np.pi*m2*np.where(k >= 0, k, 0)[None, :]/D
        v = (k >= 0)[None, :]
        return np.cos(ang)*v, np.sin(ang)*v
    def fwd_pair(k, first):
        C, Sn = cs(k)
        sg = np.where(k % 5 == first, -1.0, 1.0)[None, :] * S1
        M = np.zeros((256, 256))
        M[:128, :128] = C; M[:128, 128:] = -Sn
        M[128:, :128] = sg*Sn; M[128:, 128:] = sg*C
        return M
    MA = fwd_pair(kA, 1); MB = fwd_pair(kB, 2)
    C, Sn = cs(kC)
    MC = C.copy()
    MC[:, 65:] = -Sn[:, 1:64]
    norm = 1.0/(S*D)
    def inv_pair(k, first):
        C, Sn = cs(k)
        w = 2.0*norm
        sg = np.where(k % 5 == first, 1.0, -1.0)[None, :] * S1
        N = np.zeros((256, 256))
        N[:128, :128] = (w*C).T; N[128:, :128] = (-w*Sn).T
        N[:128, 128:] = (w*sg*Sn).T; N[128:, 128:] = (w*sg*C).T
        return N
    NA = inv_pair(kA, 1); NB = inv_pair(kB, 2)
    w = np.where((kC == 0) | (kC == 320), 1.0, 2.0)[None, :]*norm
    NC = (w*C).T.copy()
    NC[65:, :] = (-w*Sn).T[1:64, :]
    return MA, MB, MC, NA, NB, NC

def col_mats():
    k2 = np.arange(64)[:, None]; n2 = np.arange(64)[None, :]
    Gf = np.zeros((32, 128, 128))
    for k1 in range(32):
        ang = -2*np.pi*((n2*(k1 + 32*k2)) % S)/S
        gr, gi = np.cos(ang), np.sin(ang)
        Gf[k1, :64, :64] = gr; Gf[k1, :64, 64:] = -gi
        Gf[k1, 64:, :64] = gi; Gf[k1, 64:, 64:] = gr
    Gi = Gf.transpose(0, 2, 1).copy()
    return Gf, Gi


RT = float(np.sqrt(0.5)); R54 = float(np.sqrt(5)/4); RHO = float(RHO)
def cmul_const(z, ang_num, ang_den, sign):
    x, y = z
    n = (ang_num * 8) % (8*ang_den)
    if ang_num % ang_den == 0: return z
    if (ang_num * 4) % ang_den == 0:
        q = ((ang_num * 4) // ang_den) % 4
        q = q if sign > 0 else (-q) % 4
        if q == 1: return (-y, x)
        if q == 2: return (-x, -y)
        if q == 3: return (y, -x)
    if (ang_num * 8) % ang_den == 0:
        o = ((ang_num * 8) // ang_den) % 8
        o = o if sign > 0 else (-o) % 8
        c = 1 if o in (1, 7) else -1
        d = 1 if o in (1, 3) else -1
        if c == 1 and d == 1: return ((x - y) * RT, (x + y) * RT)
        if c == 1 and d == -1: return ((x + y) * RT, (y - x) * RT)
        if c == -1 and d == 1: return ((x + y) * (-RT), (x - y) * RT)
        return ((y - x) * RT, (x + y) * (-RT))
    ang = sign * 2*np.pi*ang_num/ang_den
    c, d = float(np.cos(ang)), float(np.sin(ang))
    return (x*c - y*d, x*d + y*c)

def cadd(a, b): return (a[0]+b[0], a[1]+b[1])
def csub(a, b): return (a[0]-b[0], a[1]-b[1])
def rot(t, u, sign):
    if sign > 0:
        return (t[0]-u[1], t[1]+u[0]), (t[0]+u[1], t[1]-u[0])
    return (t[0]+u[1], t[1]-u[0]), (t[0]-u[1], t[1]+u[0])

def radix4(z, sign):
    t0, t1, t2, t3 = cadd(z[0], z[2]), csub(z[0], z[2]), cadd(z[1], z[3]), csub(z[1], z[3])
    s1, s3 = rot(t1, t3, sign)
    return [cadd(t0, t2), s1, csub(t0, t2), s3]

def radix8(z, sign):
    u = [cadd(z[b], z[b+4]) for b in range(4)]
    v = [csub(z[b], z[b+4]) for b in range(4)]
    ev = radix4(u, sign)
    v1 = cmul_const(v[1], 1, 8, sign); v3 = cmul_const(v[3], 3, 8, sign)
    t0, t1 = rot(v[0], v[2], sign)
    t2, t3 = cadd(v1, v3), csub(v1, v3)
    s1, s3 = rot(t1, t3, sign)
    od = [cadd(t0, t2), s1, csub(t0, t2), s3]
    out = []
    for j in range(4): out += [ev[j], od[j]]
    return out

def lane_sel_mask(src, s, lane8):
    m = None; l = 0
    while l < 128:
        if src[l] == s:
            r = l
            while r < 128 and src[r] == s: r += 1
            t = (lane8 >= l) & (lane8 < r)
            m = t if m is None else (m | t)
            l = r
        else: l += 1
    return m


H, DH, WIN = 32, 20, 256
NB = S // 128
NEG = -1e30
QSCALE = float((DH ** -0.5) * np.log2(np.e))


def head_geom(h):
    c0 = DH*h; t = c0//128
    straddle = (c0+DH-1)//128 != t
    base = 128*t + (64 if straddle else 0)
    a = (c0//16)*16; off = c0 - a
    return c0, base, a, off


def merge_streams(streams):
    items = []
    for si, st in enumerate(streams):
        n = len(st)
        for j, f in enumerate(st):
            items.append(((j + 0.5) / n, si, j, f))
    items.sort(key=lambda t: (t[0], t[1]))
    for _, _, _, f in items:
        f()


def pack_rows(a):
    u = np.ascontiguousarray(a.astype(BF)).view(np.uint16).astype(np.uint32)
    return u[..., 0::2, :] | (u[..., 1::2, :] << np.uint32(16))


def a_consts(MPARTS):
    kA, kB, kC, a_src, b_src, c_src, gidx = lane_layout()
    MA, MB, MC, NA, NB_, NC = row_mats(); Gf, Gi = col_mats()
    M = pack_rows(np.concatenate([MA, MB, np.concatenate([MC, np.zeros((128, 128))], 1)], 0))
    N = pack_rows(np.concatenate([NA, NB_, np.concatenate([NC, np.zeros((128, 128))], 1)], 0))
    nr = 64 // MPARTS
    perm = np.concatenate([np.concatenate([np.arange(p*nr, (p+1)*nr), 64 + np.arange(p*nr, (p+1)*nr)]) for p in range(MPARTS)])
    Gi = Gi[:, perm, :]
    gi8 = np.zeros((8, 128), np.int32); gi8[:3] = gidx
    return M, N, pack_rows(Gf), pack_rows(Gi), gi8, (a_src, b_src, c_src)


def full_kernel(xa_hbm, wr_hbm, wi_hbm, x_hbm, wqkv_hbm, wo_hbm, gi_hbm, M_hbm, N_hbm, Gf_hbm, Gi_hbm, o_hbm,
                xa_ref, wr_ref, wi_ref, M_ref, N_ref, Gf_ref, Gi_ref, Wp_ref, Sf_ref, Yb_ref, Rb_ref, ya_ref,
                xraw_ref, wraw_ref, woraw_ref,
                x_ref, wk_ref, wo_ref, gi_ref, wT_ref, qT_ref, vT_ref, kw_ref, ks_ref, oT_ref, y_ref, sems,
                *, srcs, G=4, plan=None, UF=1, scopes=0, order='fine', LAG=1, online=True, QB=32, kplan=(4.4, 9.4), I1R=128, QVPAIR=False, bar1=2, bar2=4, late_out=False, split_last=True, MPARTS=2, MLAG=1, MSPLIT=True, qv_first=False, out_mode=0, QVN=1, OUTN=5, out_prep=True):
    a_src, b_src, c_src = srcs
    Tf_ref = Sf_ref
    x_u, wk_u, wo_u = x_ref, wk_ref, wo_ref
    qT_u, vT_u, kw_u, ks_u, Yb_u, Rb_u, wT_u = (r.bitcast(U32) for r in (qT_ref, vT_ref, kw_ref, ks_ref, Yb_ref, Rb_ref, wT_ref))

    nsem = [0]
    def group(pairs):
        s = sems.at[nsem[0]]; nsem[0] += 1
        return [pltpu.make_async_copy(a, b, s) for a, b in pairs]
    def start(g):
        for c in g: c.start()
    def wait(g):
        for c in g: c.wait()
    def rows_in(src, dst, r0, n):
        return [(src.at[pl.ds(r0, n), :], dst.at[pl.ds(r0, n), :])]
    def cols_in(j):
        return [(wqkv_hbm.at[:, pl.ds(D*j, D)], wraw_ref.at[j])]
    xchunks = ((0, 128), (128, 256), (384, 512), (896, 512), (1408, 640))
    x_in = [rows_in(x_hbm, xraw_ref, r0, n) for r0, n in xchunks]
    g0 = group(x_in[0] + cols_in(1))
    g1 = group(x_in[1]); g2 = group(x_in[2])
    g4 = group(cols_in(0) + cols_in(2))
    g6 = group([(wo_hbm, woraw_ref), (M_hbm, M_ref), (xa_hbm, xa_ref)])
    g7 = group(x_in[3] + x_in[4] + [(wr_hbm, wr_ref), (wi_hbm, wi_ref), (gi_hbm, gi_ref), (Gf_hbm, Gf_ref), (Gi_hbm, Gi_ref), (N_hbm, N_ref)])
    out_sem = sems.at[nsem[0]]; nsem[0] += 1
    out_copies = []
    written = {0: set(), D: set()}
    def out_dma(src_ref, r0, n, col0):
        assert all(b in written[col0] for b in range(r0//128, (r0+n)//128)), (r0, n, col0)
        for t in range(5):
            c = pltpu.make_async_copy(src_ref.at[t, pl.ds(r0, n), :], o_hbm.at[pl.ds(r0, n), pl.ds(col0 + 128*t, 128)], out_sem)
            c.start(); out_copies.append(c)

    sub8 = iota(I32, (8, 128), 0); lane8 = iota(I32, (8, 128), 1)
    zero8 = jnp.zeros((8, 128), U32)

    def xrows(i):
        return jnp.concatenate([bc(x_u[t, pl.ds(i*64, 64), :], BF) for t in range(5)], axis=1)

    def proj_pieces(i, pair=False):
        def kpiece(t):
            def f():
                kt = dot(xrows(i), bc(wk_u[t], BF))
                kw_ref[2*t, pl.ds(i*128, 128), :] = kt.astype(BF)
                ku = kw_u[2*t, pl.ds(i*64, 64), :]
                if QB == 64:
                    kr = pltpu.roll(ku, 64, 1)
                    ks_u[1, 2*t, pl.ds(i*64, 64), :] = kr
                    if t >= 1:
                        lo = iota(I32, (64, 128), 1) < 64
                        kw_u[2*t-1, pl.ds(i*64, 64), :] = jnp.where(lo, ks_u[1, 2*t-2, pl.ds(i*64, 64), :], kr)
                        ks_u[1, 2*t-1, pl.ds(i*64, 64), :] = jnp.where(lo, ku, kw_u[2*t-2, pl.ds(i*64, 64), :])
                else:
                    rot = [ku] + [pltpu.roll(ku, 32*j, 1) for j in (1, 2, 3)]
                    for j in (1, 2, 3): ks_u[j, 2*t, pl.ds(i*64, 64), :] = rot[j]
                    if t >= 1:
                        ln = iota(I32, (64, 128), 1)
                        for j in range(4):
                            jj = (j + 2) % 4
                            prev = kw_u[2*t-2, pl.ds(i*64, 64), :] if jj == 0 else ks_u[jj, 2*t-2, pl.ds(i*64, 64), :]
                            cond = ((ln >= 32*j) & (ln < 32*j + 64)) if j < 2 else ((ln >= 32*j) | (ln < 32*j - 64))
                            v = jnp.where(cond, prev, rot[jj])
                            if j == 0: kw_u[2*t-1, pl.ds(i*64, 64), :] = v
                            else: ks_u[j, 2*t-1, pl.ds(i*64, 64), :] = v
            return f
        def qvpiece(r, n):
            def f():
                o = nt_dot(jnp.concatenate([bc(wT_u[t, pl.ds(r*64, n*64), :], BF) for t in range(5)], axis=1), xrows(i))
                for u in range(n):
                    ou = o[u*128:(u+1)*128]
                    if r + u < 5:
                        qT_ref[i, (r+u)*128:(r+u+1)*128, :] = (ou * QSCALE).astype(BF)
                    else:
                        vT_ref[i, (r+u-5)*128:(r+u-4)*128, :] = ou.astype(BF)
            return f
        def qvpair(r):
            def f():
                xx = jnp.concatenate([xrows(i), xrows(i+1)], axis=0)
                o = nt_dot(jnp.concatenate([bc(wT_u[t, pl.ds(r*64, 64), :], BF) for t in range(5)], axis=1), xx)
                for u in range(2):
                    ou = o[:, u*128:(u+1)*128]
                    if r < 5: qT_ref[i+u, r*128:(r+1)*128, :] = (ou * QSCALE).astype(BF)
                    else: vT_ref[i+u, (r-5)*128:(r-4)*128, :] = ou.astype(BF)
            return f
        if pair: return [qvpair(r) for r in range(10)]
        return [kpiece(t) for t in range(5)], [qvpiece(r, QVN) for r in range(0, 10, QVN)]

    def qwin(i, h):
        c0, base, a, off = head_geom(h)
        q0 = qT_u[i, a//2:a//2+8, :]; q1 = qT_u[i, a//2+8:a//2+16, :]
        o2 = off//2
        q0 = jnp.where(sub8 >= o2, q0, zero8)
        q1 = jnp.where(sub8 < o2 + 2, q1, zero8)
        return q0, q1, (a - base)//16
    def W_from(parts):
        return bc(jnp.concatenate([parts.get(j, zero8) for j in range(8)], axis=0), BF)
    def lanemask(h):
        c0, base, a, off = head_geom(h)
        A = c0 - base
        if A + DH <= 64: return lane8 < 64
        if A >= 64: return lane8 >= 64
        return (lane8 >= 32) & (lane8 < 96)
    def qk(i, h):
        c0, base, a, off = head_geom(h)
        w = base // 64
        q0, q1, p = qwin(i, h)
        d = sub8 - lane8
        def kblk(ref, j, r0, n): return ref[w, pl.ds(j*64 + r0, n), :]
        res = []
        W1 = W_from({p: q0, p+1: q1})
        if i >= 1:
            res.append(dot(bc(kblk(kw_u, i-1, 0, 64), BF), W1))
        if i >= 2 and QB == 64:
            ks1 = ks_u.at[1]
            lo = lane8 < 64
            W2 = W_from({p: jnp.where(lo, q0, zero8), p+1: jnp.where(lo, q1, zero8),
                         (p+4) % 8: jnp.where(lo, zero8, q0), (p+5) % 8: jnp.where(lo, zero8, q1)})
            lm = lanemask(h)
            l12 = [jnp.where(lm, kblk(kw_u, i-2, j*8, 8), kblk(ks1, i, j*8, 8)) for j in range(8)]
            l3 = [jnp.where(lm, kblk(kw_u, i, j*8, 8), kblk(ks1, i-2, 32 + j*8, 8)) for j in range(4)]
            s = dot(bc(jnp.concatenate(l12 + l3, axis=0), BF), W2)
            mg = []
            for j in range(8):
                cond = (d + 8*j > 0) | (lane8 >= 64)
                mg.append(jnp.where(cond, s[8*j:8*j+8], s[128+8*j:128+8*j+8]))
            for j in range(8, 16):
                cond = (d + 8*j > 0) & (lane8 >= 64)
                mg.append(jnp.where(cond, s[128+8*(j-8):128+8*(j-8)+8], s[8*j:8*j+8]))
            res.append(jnp.concatenate(mg, axis=0))
        elif i >= 2:
            A0 = c0 - base - 6
            def inset(j):
                lo_, hi_ = (A0 + 32*j) % 128, (A0 + 32*j) % 128 + 32
                return ((lane8 >= lo_) & (lane8 < hi_)) if hi_ <= 128 else ((lane8 >= lo_) | (lane8 < hi_ - 128))
            msk = [inset(j) for j in range(3)]
            parts = {}
            for j in range(4):
                qm = (lane8 >= 32*j) & (lane8 < 32*j + 32)
                parts[(p + 2*j) % 8] = jnp.where(qm, q0, zero8)
                parts[(p + 2*j + 1) % 8] = jnp.where(qm, q1, zero8)
            W2 = W_from(parts)
            def krot(j, blk, r0):
                ref = kw_u if j == 0 else ks_u.at[j]
                return kblk(ref, blk, r0, 8)
            def compose(a):
                return jnp.where(msk[0], a[0], jnp.where(msk[1], a[1], jnp.where(msk[2], a[2], a[3])))
            la = [compose([krot(j, i-2 if j <= v // 2 else i, v*8) for j in range(4)]) for v in range(8)]
            lb = [compose([krot(j, i, 16*j + v*8) for j in range(4)]) for v in range(2)]
            s = dot(bc(jnp.concatenate(la + lb, axis=0), BF), W2)
            mg = []
            for v in range(16):
                ci = v // 4
                cond = (lane8 >= 32*ci) & (lane8 < 32*ci + 32) & (d + 8*v <= 0)
                mg.append(jnp.where(cond, s[128 + 8*(v % 4):128 + 8*(v % 4) + 8], s[8*v:8*v+8]))
            res.append(jnp.concatenate(mg, axis=0))
        else:
            s = dot(bc(kblk(kw_u, i, 0, 64), BF), W1)
            mg = [jnp.where(d + 8*j > 0, NEG, s[8*j:8*j+8]) for j in range(16)]
            res.append(jnp.concatenate(mg, axis=0))
        return res
    m_new = iota(I32, (128, 128), 0) <= iota(I32, (128, 128), 1)
    def softmax(i, ss):
        if online and len(ss) == 2:
            m1 = jnp.max(ss[0], axis=0, keepdims=True)
            p1 = jnp.exp2(ss[0] - m1).astype(BF)
            m2 = jnp.maximum(m1, jnp.max(ss[1], axis=0, keepdims=True))
            p2 = jnp.exp2(ss[1] - m2)
            alpha = jnp.exp2(m1 - m2)
            if i >= 2:
                return [(i-1, p1, alpha), (i-2, jnp.where(m_new, 0.0, p2).astype(BF), None), (i, jnp.where(m_new, p2, 0.0).astype(BF), None)]
            return [(0, p1, alpha), (1, p2.astype(BF), None)]
        m = ss[0]
        for s in ss[1:]: m = jnp.maximum(m, s)
        m = jnp.max(m, axis=0, keepdims=True)
        ps = [jnp.exp2(s - m) for s in ss]
        if i >= 2:
            return [(i-1, ps[0].astype(BF), None), (i-2, jnp.where(m_new, 0.0, ps[1]).astype(BF), None), (i, jnp.where(m_new, ps[1], 0.0).astype(BF), None)]
        if i == 1:
            return [(0, ps[0].astype(BF), None), (1, ps[1].astype(BF), None)]
        return [(0, ps[0].astype(BF), None)]
    ones8 = jnp.full((8, 128), 0x3F803F80, U32)
    def pv(i, h, pl_):
        c0, base, a, off = head_geom(h)
        ones_lo = off >= 8
        acc = None
        for j, p, alpha in pl_:
            v0 = vT_u[j, a//2:a//2+8, :]; v1 = vT_u[j, a//2+8:a//2+16, :]
            if ones_lo: v0 = jnp.where(sub8 < 4, ones8, v0)
            else: v1 = jnp.where(sub8 >= 4, ones8, v1)
            o = dot(bc(jnp.concatenate([v0, v1], axis=0), BF), p)
            if alpha is not None: o = o * alpha
            acc = o if acc is None else acc + o
        l = acc[0:8] if ones_lo else acc[24:32]
        r = pltpu.reciprocal(l, approx=True)
        inv = r * (2.0 - l * r)
        return acc, inv
    def pv_pair(i, h0, get_p):
        res = {}
        for h in (h0, h0+1):
            c0, base, a, off = head_geom(h)
            acc, inv = pv(i, h, get_p(h))
            for m in range(c0 // 8, (c0 + DH + 7) // 8):
                v = acc[8*m - a: 8*m - a + 8] * inv
                if m in res: res[m] = jnp.where(sub8 < 4, res[m], v)
                else: res[m] = v
        for m, v in res.items():
            oT_ref[i % 3, pl.ds(8*m, 8), :] = v
    def att_steps():
        units = [(i, list(range(g, g+G))) for i in range(NB) for g in range(0, H, G)]
        n = len(units)
        st_s = {}; st_p = {}
        def step(gi):
            def f():
                def do_qk():
                    if gi < n:
                        i, hs = units[gi]
                        st_s[gi] = {h: qk(i, h) for h in hs}
                def do_sm_pv():
                    if 0 <= gi - 1 < n:
                        i, hs = units[gi-1]
                        sss = st_s.pop(gi-1)
                        for j in range(0, G, 2): pv_pair(i, hs[j], lambda h: softmax(i, sss.pop(h)))
                if order == "pipe3":
                    do_qk()
                    if 0 <= gi - 2 < n:
                        i, hs = units[gi-2]
                        pss = st_p.pop(gi-2)
                        for j in range(0, G, 2): pv_pair(i, hs[j], lambda h: pss.pop(h))
                    if 0 <= gi - 1 < n:
                        i, hs = units[gi-1]
                        sss = st_s.pop(gi-1)
                        st_p[gi-1] = {h: softmax(i, sss[h]) for h in hs}
                elif order == "pipe2":
                    do_qk(); do_sm_pv()
                elif order == "pipe2r":
                    do_sm_pv(); do_qk()
                elif order == "lag":
                    if 0 <= gi - LAG < n:
                        i, hs = units[gi-LAG]
                        sss = st_s.pop(gi-LAG)
                        for j in range(0, G, 2): pv_pair(i, hs[j], lambda h: softmax(i, sss.pop(h)))
                    do_qk()
                elif order == "lag3":
                    if 0 <= gi - LAG - 1 < n:
                        i, hs = units[gi-LAG-1]
                        pss = st_p.pop(gi-LAG-1)
                        for j in range(0, G, 2): pv_pair(i, hs[j], lambda h: pss.pop(h))
                    if 0 <= gi - LAG < n:
                        i, hs = units[gi-LAG]
                        sss = st_s.pop(gi-LAG)
                        st_p[gi-LAG] = {h: softmax(i, sss[h]) for h in hs}
                    do_qk()
                elif order == "fine":
                    for j in range(0, G, 2):
                        if 0 <= gi - 1 < n:
                            i, hs = units[gi-1]
                            sss = st_s[gi-1]
                            pv_pair(i, hs[j], lambda h: softmax(i, sss.pop(h)))
                        if gi < n:
                            i, hs = units[gi]
                            st_s.setdefault(gi, {})
                            for h in hs[j:j+2]: st_s[gi][h] = qk(i, h)
            return f
        return [step(gi) for gi in range(n + LAG + 2)]

    def out_pieces(i):
        ot = {}
        def prep():
            for u in range(5):
                ot[u] = oT_ref[i % 3, pl.ds(u*128, 128), :].astype(BF).T
        def npiece(t, n):
            def f():
                if t == 0 and not out_prep: prep()
                o = jnp.concatenate([ot[u] for u in range(5)], axis=1)
                w = jnp.concatenate([wo_u[t+v] for v in range(n)], axis=1) if n > 1 else wo_u[t]
                y = dot(o, bc(w, BF))
                for v in range(n):
                    y_ref[t+v, pl.ds(i*128, 128), :] = y[:, v*128:(v+1)*128].astype(BF)
                if t + n == 5: written[D].add(i)
            return f
        return ([prep] if out_prep else []) + [npiece(t, min(OUTN, 5-t)) for t in range(0, 5, OUTN)]

    def out_kpieces(i):
        acc = [None]
        def kp(t):
            def f():
                o = oT_ref[i % 3, pl.ds(t*128, 128), :].astype(BF).T
                w = jnp.concatenate([wo_u[v, pl.ds(t*64, 64), :] for v in range(5)], axis=1)
                y = dot(o, bc(w, BF))
                acc[0] = y if acc[0] is None else acc[0] + y
                if t == 4:
                    for v in range(5):
                        y_ref[v, pl.ds(i*128, 128), :] = acc[0][:, v*128:(v+1)*128].astype(BF)
                    written[D].add(i)
            return f
        return [kp(t) for t in range(5)]

    def wprep_pieces():
        def piece(j, arr):
            def f():
                ref = (wr_ref, wi_ref)[arr]
                gidx = [jnp.broadcast_to(gi_ref[t:t+1, :], (8, 128)) for t in range(3)]
                mA0, mA1 = lane_sel_mask(a_src, 0, lane8), lane_sel_mask(a_src, 1, lane8)
                mB0, mB1 = lane_sel_mask(b_src, 0, lane8), lane_sel_mask(b_src, 1, lane8)
                mC0, mC1 = lane_sel_mask(c_src, 0, lane8), lane_sel_mask(c_src, 1, lane8)
                cols = slice(128*j, 128*j+128)
                t2 = jnp.concatenate([ref[256:321, cols], jnp.zeros((63, 128), BF)], axis=0)
                tiles = [bc(ref[0:128, cols].T, U32), bc(ref[128:256, cols].T, U32), bc(t2.T, U32)]
                for v in range(8):
                    u = 8*j + v
                    g = [jnp.take_along_axis(tiles[t][8*v:8*v+8], gidx[t], axis=1) for t in range(3)]
                    pos = 17*(u//2) + 8*(u % 2)
                    Wp_ref[arr, 0, pos:pos+8, :] = jnp.where(mA0, g[0], jnp.where(mA1, g[1], g[2]))
                    Wp_ref[arr, 1, pos:pos+8, :] = jnp.where(mB0, g[0], jnp.where(mB1, g[1], g[2]))
                    Wp_ref[arr, 2, pos:pos+8, :] = jnp.where(mC0, g[0], jnp.where(mC1, g[1], g[2]))
            return f
        return [piece(j, arr) for j in range(16) for arr in range(2)]

    def f1_pieces(UF):
        nr = 16*UF
        def piece(b, g):
            def f():
                def dft5(r0):
                    T = [xa_ref[pl.ds(r0, 16), t*128:(t+1)*128].astype(F32) for t in range(5)]
                    p, q, r, w = T[1]+T[4], T[2]+T[3], T[1]-T[4], T[2]-T[3]
                    u = p+q
                    t1 = T[0] - 0.25*u; t2 = (p-q)*R54
                    return [(T[0]+u).astype(BF), (t1+t2).astype(BF), (r + RHO*w).astype(BF),
                            (t1-t2).astype(BF), (RHO*r - w).astype(BF)]
                chunks = [dft5(64*(8*a+b) + nr*g + 16*c) for a in range(4) for c in range(UF)]
                U0, a1, b1, a2, b2 = (jnp.concatenate([ch[j] for ch in chunks], axis=0) for j in range(5))
                RA = dot(jnp.concatenate([a1, b1], axis=1), bc(M_ref[0:128, :], BF))
                RB = dot(jnp.concatenate([a2, b2], axis=1), bc(M_ref[128:256, :], BF))
                RC = dot(U0, bc(M_ref[256:320, 0:128], BF))
                ln = iota(I32, RC.shape, 1)
                RCi = jnp.where((ln == 0) | (ln == 64), 0.0, pltpu.roll(RC, 64, 1))
                for P, (Rr, Ri) in enumerate(((RA[:, 0:128], RA[:, 128:256]), (RB[:, 0:128], RB[:, 128:256]), (RC, RCi))):
                    z = [(Rr[nr*a:nr*a+nr], Ri[nr*a:nr*a+nr]) for a in range(4)]
                    Sx = radix4(z, -1)
                    for ka in range(4):
                        x, y = cmul_const(Sx[ka], b*ka, 32, -1)
                        Sf_ref[P, 0, ka, b, nr*g:nr*g+nr, :] = x
                        Sf_ref[P, 1, ka, b, nr*g:nr*g+nr, :] = y
            return f
        return [piece(b, g) for g in range(4//UF) for b in range(8)]

    def f2_pieces():
        def piece(ka, g, P):
            def f():
                z = [(Sf_ref[P, 0, ka, b, 16*g:16*g+16, :], Sf_ref[P, 1, ka, b, 16*g:16*g+16, :]) for b in range(8)]
                o = radix8(z, -1)
                for kb in range(8):
                    k1 = ka + 4*kb
                    Yb_ref[k1, P, 16*g:16*g+16, :] = o[kb][0].astype(BF)
                    Yb_ref[k1, P, 64+16*g:64+16*g+16, :] = o[kb][1].astype(BF)
            return f
        return [[piece(ka, g, P) for ka in range(4) for P in range(3)] for g in range(4)]

    def m_pieces():
        def m1(be, P, als):
            def f():
                for al in als:
                    k1 = be + 8*al
                    X = dot(bc(Gf_ref[k1], BF), bc(Yb_u[k1, P], BF))
                    wr = Wp_ref[0, P, pl.ds(k1//2, 64, stride=17), :]
                    wi = Wp_ref[1, P, pl.ds(k1//2, 64, stride=17), :]
                    if k1 % 2 == 0:
                        wr = bc(wr << 16, F32); wi = bc(wi << 16, F32)
                    else:
                        wr = bc(wr & jnp.uint32(0xFFFF0000), F32); wi = bc(wi & jnp.uint32(0xFFFF0000), F32)
                    for c in range(4):
                        rs = slice(16*c, 16*c + 16)
                        xr, xi = X[16*c:16*c+16], X[64+16*c:64+16*c+16]
                        Yb_ref[k1, P, 16*c:16*c+16, :] = (xr*wr[rs] - xi*wi[rs]).astype(BF)
                        Yb_ref[k1, P, 64+16*c:64+16*c+16, :] = (xr*wi[rs] + xi*wr[rs]).astype(BF)
            return f
        def m2(be, P, part):
            nr = 64 // MPARTS
            def f():
                V = []
                for al in range(4):
                    k1 = be + 8*al
                    Vv = dot(bc(Gi_ref[k1, pl.ds(part*nr, nr), :], BF), bc(Yb_u[k1, P], BF))
                    V.append((Vv[0:nr], Vv[nr:2*nr]))
                Tn = radix4(V, +1)
                for na in range(4):
                    x, y = cmul_const(Tn[na], be*na, 32, +1)
                    Tf_ref[P, 0, na, be, pl.ds(part*nr, nr), :] = x
                    Tf_ref[P, 1, na, be, pl.ds(part*nr, nr), :] = y
            return f
        units = [(be, P) for P in range(3) for be in range(8)]
        out = []; done = []
        for n_ in range(len(units) + MLAG):
            if n_ < len(units):
                if MSPLIT: out += [m1(*units[n_], (0, 1)), m1(*units[n_], (2, 3))]
                else: out.append(m1(*units[n_], (0, 1, 2, 3)))
            if n_ - MLAG >= 0:
                out += [m2(*units[n_-MLAG], part) for part in range(MPARTS)]
                if units[n_-MLAG][0] == 7: done.append(len(out))
        return out, done

    def i2_pieces():
        def piece(na, g, P):
            def f():
                z = [(Tf_ref[P, 0, na, be, 16*g:16*g+16, :], Tf_ref[P, 1, na, be, 16*g:16*g+16, :]) for be in range(8)]
                o = radix8(z, +1)
                ln = iota(I32, (16, 128), 1)
                for nb in range(8):
                    n1 = na + 4*nb
                    rows = slice(64*n1+16*g, 64*n1+16*g+16)
                    if P < 2:
                        Rb_ref[2*P, rows, :] = o[nb][0].astype(BF)
                        Rb_ref[2*P+1, rows, :] = o[nb][1].astype(BF)
                    else:
                        Rb_ref[4, rows, :] = jnp.where(ln <= 64, o[nb][0], pltpu.roll(o[nb][1], 64, 1)).astype(BF)
            return f
        return [[piece(na, g, P) for g in range(4) for na in range(4)] for P in range(3)]

    def i1_pieces(R=128):
        def piece(j):
            def f():
                rows = slice(R*j, R*(j+1))
                def rb(t): return bc(Rb_u[t, pl.ds(R*j//2, R//2), :], BF)
                EA = dot(jnp.concatenate([rb(0), rb(1)], axis=1), bc(N_ref[0:128, :], BF))
                EB = dot(jnp.concatenate([rb(2), rb(3)], axis=1), bc(N_ref[128:256, :], BF))
                U0 = dot(rb(4), bc(N_ref[256:320, 0:128], BF))
                e1, f1, e2, f2 = EA[:, :128], EA[:, 128:], EB[:, :128], EB[:, 128:]
                u = e1+e2
                t1 = U0 - 0.25*u; t2 = (e1-e2)*R54
                al, be = t1+t2, t1-t2
                ga = f1 + RHO*f2; de = RHO*f1 - f2
                ys = [U0+u, al-ga, be-de, be+de, al+ga]
                for t in range(5):
                    ya_ref[t, rows, :] = ys[t].astype(BF)
                if (R*(j+1)) % 128 == 0: written[0].add(R*(j+1)//128 - 1)
            return f
        return [piece(j) for j in range(S // R)]

    for g in (g0, g1, g2, g4, g6, g7): start(g)
    def retile(src, dst, r0, n):
        for t in range(5):
            dst[t, pl.ds(r0//2, n//2), :] = bc(src[pl.ds(r0, n), t*128:(t+1)*128], U32)
    def transposes(j, r0):
        for r in range(5):
            for c in range(5):
                wT_ref[r, r0 + c*128:r0 + (c+1)*128, :] = wraw_ref[j, r*128:(r+1)*128, c*128:(c+1)*128].T
    def kblocks(i0, i1):
        for i in range(i0, i1):
            retile(xraw_ref, x_ref, 128*i, 128)
            for f in proj_pieces(i)[0]: f()
    def scope(name):
        return jax.named_scope(name) if scopes else contextlib.nullcontext()
    with scope("p0w"): wait(g0)
    with scope("p0"):
        retile(wraw_ref.at[1], wk_ref, 0, D)
        kblocks(0, 1)
    with scope("p1w"): wait(g1)
    with scope("p1"): kblocks(1, 3)
    with scope("p2w"): wait(g2)
    with scope("p2"): kblocks(3, 7)
    with scope("p4w"): wait(g4)
    with scope("p4"):
        transposes(0, 0); transposes(2, 640)
        for f in proj_pieces(0)[1]: f()

    GPB = H // G
    items = []
    def place(lst, lo, hi, prio):
        n = len(lst)
        for j, fn in enumerate(lst):
            items.append((lo + (hi - lo) * (j + 0.5) / n, prio, len(items), fn))
    def at(key, fn): items.append((key, -1, len(items), fn))
    for gi, fn in enumerate(att_steps()):
        items.append((gi + 0.5, 0, len(items), fn))
    if QVPAIR:
        for sl in range(NB - 1):
            i = sl + 1
            if i + 1 < NB:
                lst = proj_pieces(i, True)[:5] if sl % 2 == 0 else proj_pieces(i, True)[5:]
            else:
                lst = proj_pieces(i)[1][:5]
            if sl == 0: lst = lst + proj_pieces(1)[1][5:]
            place(lst, GPB*sl, GPB*(sl+1) + (0.4 if sl % 2 == 0 else -0.5), 1)
    else:
        for i in range(1, NB):
            place(proj_pieces(i)[1], GPB*(i-1), GPB*i + 0.4, 1)
    klo, khi = kplan
    for i in range(7, NB):
        def rt(i=i): retile(xraw_ref, x_ref, 128*i, 128)
        a_ = klo + (khi - klo) * (i - 7) / 9
        place([rt] + proj_pieces(i)[0], GPB*a_, GPB*min(a_ + (khi - klo) / 9, i - 0.6), 1)
    for i in range(NB):
        if i == 0:
            place(out_pieces(i), GPB*bar1 + 0.1, GPB*bar1 + 0.2*(GPB*3 - GPB*bar1) + 0.2, 2)
        elif i == 1:
            place(out_pieces(i), GPB*bar1 + 0.3, GPB*3 + LAG + 1, 2)
        elif late_out and i == NB-3:
            place(out_pieces(i), GPB*(NB-1) - 1, GPB*(NB-1) + 2, 2)
        elif late_out and i == NB-2:
            place(out_pieces(i), GPB*(NB-1) + 4, GPB*(NB-1) + 6, 2)
        elif split_last and i == NB-1:
            for t, fn in enumerate(out_kpieces(i)):
                hl = min(H-1, (128*t + 127)//DH)
                at(GPB*i + hl//G + LAG + 0.6, fn)
        elif out_mode == 0:
            place(out_pieces(i), GPB*(i+1) + LAG + 1, GPB*(i+2) + LAG + 1 if i < NB-1 else GPB*(i+1) + LAG + 2, 2)
        elif out_mode == 1:
            place(out_pieces(i), GPB*(i+1) + 2, GPB*(i+1) + 2.01, 2)
    P_ = plan or dict(f1=(2, 6.0), wp=(4.3, 5.8), m=(6.5, 11.6), i1=(12.0, 14.2))
    lo, hi = GPB*P_["f1"][0], GPB*P_["f1"][1]
    place(f1_pieces(UF), lo, hi, 3)
    q_ = (hi - lo) / 4
    f2e = GPB*P_["m"][0]
    for g, lst in enumerate(f2_pieces()):
        place(lst, lo + q_*(g+1) + 0.01, min(lo + q_*(g+2), f2e) if g < 3 else f2e, 5)
    place(wprep_pieces(), GPB*P_["wp"][0], GPB*P_["wp"][1], 4)
    mlist, mdone = m_pieces()
    lo, hi = GPB*P_["m"][0], GPB*P_["m"][1]
    place(mlist, lo, hi, 3)
    keys = [lo + (hi - lo) * d_ / len(mlist) + 0.01 for d_ in mdone] + [GPB*P_["i1"][0]]
    for P, lst in enumerate(i2_pieces()):
        place(lst, keys[P], keys[P+1] if P < 2 else keys[3], 5)
    place(i1_pieces(I1R), GPB*P_["i1"][0], GPB*P_["i1"][1], 3)
    y1 = 128*(bar2-2)
    def sync(waits=(), outs=(), starts=(), pre=None):
        def f():
            for g in starts: start(g)
            for g in waits: wait(g)
            for o in outs: out_dma(*o)
            if pre: pre()
        return f
    at(GPB*bar1 - 0.01, sync(waits=(g6,), pre=lambda: retile(woraw_ref, wo_ref, 0, D)))
    at(GPB*bar2 + LAG + 1.01, sync(waits=(g7,), outs=((y_ref, 0, y1, D),)))
    at(GPB*14 + LAG + 1.01, sync(outs=((y_ref, y1, 1664 - y1, D), (ya_ref, 0, S, 0))))
    at(GPB*18, sync(outs=((y_ref, 1664, 384, D),)))
    items.sort(key=lambda t: t[:3])
    if scopes:
        for sl, grp in itertools.groupby(items, key=lambda t: int(t[0] // (GPB*scopes))):
            with jax.named_scope("slot%02d" % sl):
                for it in grp: it[3]()
    else:
        for it in items: it[3]()
    with scope("zztail"):
        for c in out_copies: c.wait()
    assert nsem[0] <= NSEM


NSEM = 7


def make_full(**kw):
    M, N, Gf, Gi, gi8, srcs = a_consts(kw.get('MPARTS', 2))
    def V(shape, dt): return pltpu.VMEM(shape, dt)
    def f(A_x, A_w_r, A_w_i, B_x, B_wqkv, B_wo):
        hbm = pl.BlockSpec(memory_space=pltpu.HBM)
        out = pl.pallas_call(
            functools.partial(full_kernel, srcs=srcs, **kw),
            out_shape=jax.ShapeDtypeStruct((S, 2*D), BF),
            in_specs=[hbm]*11, out_specs=hbm,
            scratch_shapes=[V((S, D), BF), V((321, S), BF), V((321, S), BF),
                            V((320, 256), U32), V((320, 256), U32),
                            V((32, 64, 128), U32), V((32, 64, 128), U32),
                            V((2, 3, 17*64, 128), U32),
                            V((3, 2, 4, 8, 64, 128), F32),
                            V((32, 3, 128, 128), BF),
                            V((5, S, 128), BF),
                            V((5, S, 128), BF),
                            V((S, D), BF), V((3, D, D), BF), V((D, D), BF),
                            V((5, S//2, 128), U32), V((5, D//2, 128), U32), V((5, D//2, 128), U32), V((8, 128), I32),
                            V((5, 1280, 128), BF),
                            V((NB, 640, 128), BF), V((NB, 640, 128), BF),
                            V((9, S, 128), BF), V((4, 9, S, 128), BF),
                            V((3, 640, 128), F32), V((5, S, 128), BF),
                            pltpu.SemaphoreType.DMA((NSEM,))],
            compiler_params=pltpu.CompilerParams(vmem_limit_bytes=110*2**20), name="fk")(
                A_x.reshape(S, D), A_w_r.T, A_w_i.T, B_x.reshape(S, D), B_wqkv, B_wo, gi8, M, N, Gf, Gi)
        return out.reshape(1, S, 2*D)
    return f


_KERNEL_FN = make_full()


@jax.jit
def pallas_concat_heads__spectral_gfnet__sliding_block__prompt_kernel(
    A_x: jax.Array,
    A_w_r: jax.Array,
    A_w_i: jax.Array,
    B_x: jax.Array,
    B_wqkv: jax.Array,
    B_wo: jax.Array,
):
    return _KERNEL_FN(A_x, A_w_r, A_w_i, B_x, B_wqkv, B_wo)
```
